```python
import jax
import jax.numpy as jnp

def _softmax(x, axis=-1):
    return jax.nn.softmax(x, axis=axis)
def _gelu(x):
    return jax.nn.gelu(x, approximate=True)
def _silu(x):
    return jax.nn.silu(x)
def _sigmoid(x):
    return jax.nn.sigmoid(x)
def _layernorm(x, axis=-1, eps=1e-5):
    m = jnp.mean(x, axis=axis, keepdims=True)
    v = jnp.var(x, axis=axis, keepdims=True)
    return (x - m) / jnp.sqrt(v + eps)
def _scatter_add(tgt, idx, src, axis=0):
    return tgt.at[idx].add(src)
def _segment_sum(src, seg, n):
    return jax.ops.segment_sum(src, seg, n)
class _Rng:
    def __init__(self, key):
        self._k = key
    def _next(self):
        self._k, sub = jax.random.split(self._k)
        return sub
    def normal(self, shape):
        return jax.random.normal(self._next(), shape, dtype=jnp.bfloat16)
    def randint(self, lo, hi, shape):
        return jax.random.randint(self._next(), shape, lo, hi, dtype=jnp.int32)
    def uniform(self, shape, lo=0.0, hi=1.0):
        return jax.random.uniform(self._next(), shape, jnp.bfloat16, lo, hi)
    def permutation(self, n):
        return jax.random.permutation(self._next(), n)


kernel_name = 'gated_mix__sliding_block_cached__moe_arch_mod__decode'

def setup_inputs():
    _rng = _Rng(jax.random.key(int.from_bytes(__import__("os").urandom(4), "little")))
    _w = (lambda a: (lambda t: t.astype(jnp.bfloat16) if jnp.issubdtype(t.dtype, jnp.floating) else t)(jnp.asarray(a)))
    def _A_setup():
        B, Sq, D = 1, 1, 640
        Hq, Hkv, Sk, Dh = 32, 32, 32768, 192
        assert Hq % Hkv == 0, (Hq, Hkv)
        return {
            "x": _w((lambda *s: _rng.normal(s) * 0.05)(B, Sq, D)),
            "k_cache": _w((lambda *s: _rng.normal(s) * 0.05)(B, Hkv, Sk, Dh)),
            "v_cache": _w((lambda *s: _rng.normal(s) * 0.05)(B, Hkv, Sk, Dh)),
            "wq": _w((lambda *s: _rng.normal(s) * 0.05)(D, Hq * Dh) * (D ** -0.5)),
            "wo": _w((lambda *s: _rng.normal(s) * 0.05)(Hq * Dh, D) * ((Hq * Dh) ** -0.5)),
        }
    _A_in = _A_setup()

    def _B_setup():
        B, S, D, F, C = 1, 1, 640, 1536, 1
        return {
            "x": _w((lambda *s: _rng.normal(s) * 0.05)(B, S, D)),
            "w_r": _w((lambda *s: _rng.normal(s) * 0.05)(D)),
            "w_gate": _w((lambda *s: _rng.normal(s) * 0.05)(D, F)),
            "w_up": _w((lambda *s: _rng.normal(s) * 0.05)(D, F)),
            "w_down": _w((lambda *s: _rng.normal(s) * 0.05)(F, D)),
        }
    _B_in = _B_setup()

    return {
        "A_x": _A_in["x"],
        "A_k_cache": _A_in["k_cache"],
        "A_v_cache": _A_in["v_cache"],
        "A_wq": _A_in["wq"],
        "A_wo": _A_in["wo"],
        "B_x": _B_in["x"],
        "B_w_r": _B_in["w_r"],
        "B_w_gate": _B_in["w_gate"],
        "B_w_up": _B_in["w_up"],
        "B_w_down": _B_in["w_down"],
        "gate_w": _w((lambda *s: _rng.normal(s) * 0.05)(640)),
    }

def reference(A_x, A_k_cache, A_v_cache, A_wq, A_wo, B_x, B_w_r, B_w_gate, B_w_up, B_w_down, gate_w):
    def _A_ref(x, k_cache, v_cache, wq, wo):
        B, Sq, D = x.shape
        Hq, Dh = 32, 192
        Hkv, Sk = k_cache.shape[1], k_cache.shape[2]
        W = min(4096, max(256, Sk // 4))
        rep = Hq // Hkv
        q = (lambda x, *d: x.transpose(*d))((x @ wq).reshape(B, Sq, Hq, Dh), 0, 2, 1, 3)
        k = jnp.repeat(k_cache[:, :, Sk - W:, :], rep, axis=1)
        v = jnp.repeat(v_cache[:, :, Sk - W:, :], rep, axis=1)
        scores = jnp.einsum("bhqd,bhkd->bhqk", q, k) * (Dh ** -0.5)
        p = _softmax(scores, axis=-1)
        o = jnp.einsum("bhqk,bhkd->bhqd", p, v)
        return (lambda x, *d: x.transpose(*d))(o, 0, 2, 1, 3).reshape(B, Sq, Hq * Dh) @ wo

    def _B_ref(x, w_r, w_gate, w_up, w_down):
        B, S, D = x.shape
        C = 1
        r = x @ w_r
        idx = jnp.argsort(-r, axis=-1)[:, :C]
        idx_e = jnp.repeat(idx.reshape(B, C, 1), D, axis=2)
        x_sel = jnp.take_along_axis(x, idx_e, axis=1)
        g = _silu(x_sel @ w_gate)
        u = x_sel @ w_up
        y = (g * u) @ w_down
        r_sel = _sigmoid(jnp.take_along_axis(r, idx, axis=1))
        y = y * r_sel.reshape(B, C, 1)
        b_off = (jnp.arange(B) * S).reshape(B, 1)
        flat_idx = (idx + b_off).reshape(B * C)
        zero = (x * 0.0).reshape(B * S, D)
        upd = _scatter_add(zero, flat_idx, y.reshape(B * C, D), axis=0)
        return x + upd.reshape(B, S, D)

    x = A_x
    g = _sigmoid((x * gate_w).sum(-1, keepdims=True))
    a = _A_ref(x, A_k_cache, A_v_cache, A_wq, A_wo)
    b = _B_ref(x, B_w_r, B_w_gate, B_w_up, B_w_down)
    return g * a + (1 - g) * b
```

```python
import functools
import jax
import jax.numpy as jnp
from jax import lax
from jax.experimental import pallas as pl
from jax.experimental.pallas import tpu as pltpu

D = 640
H = 32
DH = 192
F = 1536
G = 2
NG = H // G
GD = G * DH


def _build(NB=2, WO_CHUNKS=(4, 4, 4, 2, 1, 1), prio=True):
    assert sum(WO_CHUNKS) == NG

    def kernel(x_hbm, wr_hbm, gw_hbm, kt_hbm, vt_hbm, wq_hbm, wo_hbm, wg_hbm, wu_hbm, wd_hbm,
               out_ref,
               x_v, wr_v, gw_v, kbuf, vbuf, wq_v, wo_v, wg_v, wu_v, wd_v, q_s, o_s,
               ssem, ksem, vsem, wsem, wosem):
        SK = kt_hbm.shape[-1]
        W = kbuf.shape[-1]

        def kcp(g, slot):
            return pltpu.make_async_copy(kt_hbm.at[g, :, pl.ds(SK - W, W)], kbuf.at[slot], ksem.at[slot])

        def vcp(g, slot):
            return pltpu.make_async_copy(vt_hbm.at[g, :, pl.ds(SK - W, W)], vbuf.at[slot], vsem.at[slot])

        cx = pltpu.make_async_copy(x_hbm, x_v, ssem.at[0])
        cr = pltpu.make_async_copy(wr_hbm, wr_v, ssem.at[1])
        cg = pltpu.make_async_copy(gw_hbm, gw_v, ssem.at[2])
        cwq = pltpu.make_async_copy(wq_hbm, wq_v, wsem.at[0])
        cwg = pltpu.make_async_copy(wg_hbm, wg_v, wsem.at[1])
        cwu = pltpu.make_async_copy(wu_hbm, wu_v, wsem.at[2])
        cwd = pltpu.make_async_copy(wd_hbm, wd_v, wsem.at[3])
        wo_cps = []
        off = 0
        for j, n in enumerate(WO_CHUNKS):
            wo_cps.append(pltpu.make_async_copy(
                wo_hbm.at[pl.ds(off * GD, n * GD), :], wo_v.at[pl.ds(off * GD, n * GD), :], wosem.at[j]))
            off += n

        P1 = 1 if prio else 0
        cwg.start(); cx.start(); cr.start(); cg.start()
        cwu.start(priority=P1); cwd.start(); cwq.start(priority=P1)
        for g in range(NB):
            kcp(g, g).start()
            vcp(g, g).start(priority=P1)

        cx.wait(); cr.wait(); cg.wait()
        x = x_v[...]
        x8 = jnp.broadcast_to(x, (8, D))
        xf = x.astype(jnp.float32)
        wr = wr_v[...].astype(jnp.float32)
        gw = gw_v[...].astype(jnp.float32)
        r_acc = jnp.zeros((1, 128), jnp.float32)
        g_acc = jnp.zeros((1, 128), jnp.float32)
        for j in range(D // 128):
            xs = xf[:, j * 128:(j + 1) * 128]
            r_acc = r_acc + xs * wr[j:j + 1, :]
            g_acc = g_acc + xs * gw[j:j + 1, :]
        r_sel = jax.nn.sigmoid(jnp.sum(r_acc, axis=-1, keepdims=True))
        gate = jax.nn.sigmoid(jnp.sum(g_acc, axis=-1, keepdims=True))

        cwg.wait()
        gg = jnp.dot(x8, wg_v[...], preferred_element_type=jnp.float32)
        cwu.wait()
        uu = jnp.dot(x8, wu_v[...], preferred_element_type=jnp.float32)
        hh = (gg * jax.nn.sigmoid(gg) * uu).astype(jnp.bfloat16)
        cwd.wait()
        y = jnp.dot(hh, wd_v[...], preferred_element_type=jnp.float32)[0:1, :]
        b = xf + (xf * 0.0 + y * r_sel)
        b_scaled = (1.0 - gate) * b

        row = lax.broadcasted_iota(jnp.int32, (8, GD), 0)
        col = lax.broadcasted_iota(jnp.int32, (8, GD), 1)
        diag = (col >= row * DH) & (col < (row + 1) * DH)
        cwq.wait()
        for g in range(NG):
            qg = jnp.dot(x8, wq_v[:, g * GD:(g + 1) * GD], preferred_element_type=jnp.float32)
            q_s[g] = jnp.where(diag, qg, 0.0).astype(jnp.bfloat16)

        scale = DH ** -0.5

        def body(g, carry):
            slot = lax.rem(g, NB)
            kcp(g, slot).wait()
            s = jnp.dot(q_s[g], kbuf[slot], preferred_element_type=jnp.float32) * scale
            m = jnp.max(s, axis=-1, keepdims=True)
            p = jnp.exp(s - m)
            l = jnp.sum(p, axis=-1, keepdims=True)

            @pl.when(g + NB < NG)
            def _():
                kcp(g + NB, slot).start()

            vcp(g, slot).wait()
            o = lax.dot_general(p.astype(jnp.bfloat16), vbuf[slot], (((1,), (1,)), ((), ())),
                                preferred_element_type=jnp.float32)
            o_s[g] = jnp.where(diag, o / l, 0.0).astype(jnp.bfloat16)

            @pl.when(g + NB < NG)
            def _():
                vcp(g + NB, slot).start(priority=P1)

            @pl.when(g == NG - NB)
            def _():
                for j, c in enumerate(wo_cps):
                    c.start(priority=(j % 2) if prio else 0)
            return carry

        lax.fori_loop(0, NG, body, 0)

        acc = jnp.zeros((8, D), jnp.float32)
        off = 0
        for j, n in enumerate(WO_CHUNKS):
            wo_cps[j].wait()
            for g in range(off, off + n):
                acc = acc + jnp.dot(o_s[g], wo_v[g * GD:(g + 1) * GD, :], preferred_element_type=jnp.float32)
            off += n
        a = jnp.sum(acc, axis=0, keepdims=True)
        out_ref[...] = (gate * a + b_scaled).astype(out_ref.dtype)

    @jax.jit
    def pallas_gated_mix__sliding_block_cached__moe_arch_mod__decode_kernel(A_x, A_k_cache, A_v_cache, A_wq, A_wo, B_x, B_w_r, B_w_gate, B_w_up, B_w_down, gate_w):
        SK = A_k_cache.shape[2]
        W = min(4096, max(256, SK // 4))
        kt = jnp.swapaxes(A_k_cache, 2, 3).reshape(NG, GD, SK)
        vt = jnp.swapaxes(A_v_cache, 2, 3).reshape(NG, GD, SK)
        x = A_x.reshape(1, D)
        wr = B_w_r.reshape(D // 128, 128)
        gw = gate_w.reshape(D // 128, 128)
        bf = jnp.bfloat16
        out = pl.pallas_call(
            kernel,
            out_shape=jax.ShapeDtypeStruct((1, D), bf),
            in_specs=[pl.BlockSpec(memory_space=pl.ANY)] * 10,
            out_specs=pl.BlockSpec(memory_space=pltpu.VMEM),
            scratch_shapes=[
                pltpu.VMEM((1, D), bf), pltpu.VMEM((D // 128, 128), bf), pltpu.VMEM((D // 128, 128), bf),
                pltpu.VMEM((NB, GD, W), bf), pltpu.VMEM((NB, GD, W), bf),
                pltpu.VMEM((D, H * DH), bf), pltpu.VMEM((H * DH, D), bf),
                pltpu.VMEM((D, F), bf), pltpu.VMEM((D, F), bf), pltpu.VMEM((F, D), bf),
                pltpu.VMEM((NG, 8, GD), bf), pltpu.VMEM((NG, 8, GD), bf),
                pltpu.SemaphoreType.DMA((3,)), pltpu.SemaphoreType.DMA((NB,)), pltpu.SemaphoreType.DMA((NB,)),
                pltpu.SemaphoreType.DMA((4,)), pltpu.SemaphoreType.DMA((len(WO_CHUNKS),)),
            ],
            compiler_params=pltpu.CompilerParams(vmem_limit_bytes=100 * 1024 * 1024),
        )(x, wr, gw, kt, vt, A_wq, A_wo, B_w_gate, B_w_up, B_w_down)
        return out.reshape(1, 1, D)
    return pallas_gated_mix__sliding_block_cached__moe_arch_mod__decode_kernel


pallas_gated_mix__sliding_block_cached__moe_arch_mod__decode_kernel = _build()
```

```python
import functools
import jax
import jax.numpy as jnp
from jax import lax
from jax.experimental import pallas as pl
from jax.experimental.pallas import tpu as pltpu

D = 640
H = 32
DH = 192
F = 1536
G = 2
NG = H // G
GD = G * DH
CW = 128


def _build(D1=16, compute=True, wo_piece="row16", nobc=True, peel=True):
    def kernel(x_hbm, wr_hbm, gw_hbm, kt_hbm, vt_hbm, wq_hbm, wo_hbm, wg_hbm, wu_hbm, wd_hbm,
               out_ref,
               x_v, wr_v, gw_v, ring, wq_v, wo_v, wg_v, wu_v, wd_v, acc_s,
               ssem, rsem, qsem, osem, fsem):
        SK = kt_hbm.shape[-1]
        NC = ring.shape[0]
        W = NC * CW
        base = SK - W

        def kv_copy(src, g, j):
            return pltpu.make_async_copy(src.at[g, :, pl.ds(base + j * CW, CW)], ring.at[j], rsem.at[j])

        def mo(v, m):
            return v if isinstance(v, int) else pl.multiple_of(v, m)

        def wq_pieces(g):
            slot = g % 2
            out = []
            for c in range(3):
                for r in range(8):
                    out.append(lambda c=c, r=r: pltpu.make_async_copy(
                        wq_hbm.at[pl.ds(r * 80, 80), pl.ds(mo(g * GD + c * 128, 128), 128)],
                        wq_v.at[slot, pl.ds(r * 80, 80), pl.ds(c * 128, 128)], qsem.at[slot]))
            return out

        def wo_pieces(g):
            slot = g % 2
            out = []
            if wo_piece == "row16":
                for i in range(24):
                    out.append(lambda i=i: pltpu.make_async_copy(
                        wo_hbm.at[pl.ds(mo(g * GD + i * 16, 16), 16), :],
                        wo_v.at[slot, pl.ds(i * 16, 16), :], osem.at[slot]))
            else:
                for c in range(5):
                    for r in range(4):
                        out.append(lambda c=c, r=r: pltpu.make_async_copy(
                            wo_hbm.at[pl.ds(mo(g * GD + r * 96, 16), 96), pl.ds(c * 128, 128)],
                            wo_v.at[slot, pl.ds(r * 96, 96), pl.ds(c * 128, 128)], osem.at[slot]))
            return out

        def ffn_pieces(g):
            out = []
            for (src, dst, k) in ((wg_hbm, wg_v, 0), (wu_hbm, wu_v, 1)):
                for i in range(6):
                    def mk(src=src, dst=dst, k=k, i=i):
                        t = g * 6 + i
                        r = mo((t & 7) * 80, 16)
                        c = mo((t >> 3) * 128, 128)
                        return pltpu.make_async_copy(src.at[pl.ds(r, 80), pl.ds(c, 128)],
                                                     dst.at[pl.ds(r, 80), pl.ds(c, 128)], fsem.at[k])
                    out.append(mk)
            for i in range(6):
                def mk(i=i):
                    if wo_piece == "row16":
                        r = mo(g * 96 + i * 16, 16)
                        return pltpu.make_async_copy(wd_hbm.at[pl.ds(r, 16), :], wd_v.at[pl.ds(r, 16), :], fsem.at[2])
                    else:
                        if i == 5:
                            return None
                        r = mo(g * 96, 16)
                        return pltpu.make_async_copy(wd_hbm.at[pl.ds(r, 96), pl.ds(i * 128, 128)],
                                                     wd_v.at[pl.ds(r, 96), pl.ds(i * 128, 128)], fsem.at[2])
                out.append(mk)
            if wo_piece != "row16":
                out = out[:-1]
            return out

        cx = pltpu.make_async_copy(x_hbm, x_v, ssem.at[0])
        cr = pltpu.make_async_copy(wr_hbm, wr_v, ssem.at[1])
        cg = pltpu.make_async_copy(gw_hbm, gw_v, ssem.at[2])

        def wq_all(slot):
            return pltpu.make_async_copy(wq_v.at[slot], wq_v.at[slot], qsem.at[slot])

        def wo_all(slot):
            return pltpu.make_async_copy(wo_v.at[slot], wo_v.at[slot], osem.at[slot])

        kv_copy(kt_hbm, 0, 0).start(priority=1)
        pltpu.make_async_copy(wq_hbm.at[:, pl.ds(0, GD)], wq_v.at[0], qsem.at[0]).start(priority=0)
        cx.start()
        for j in range(1, D1):
            kv_copy(kt_hbm, 0, j).start(priority=1)
        cr.start(); cg.start()

        row = lax.broadcasted_iota(jnp.int32, (8, GD), 0)
        col = lax.broadcasted_iota(jnp.int32, (8, GD), 1)
        diag = (col >= row * DH) & (col < (row + 1) * DH)
        scale = DH ** -0.5

        cx.wait()
        x8 = jnp.broadcast_to(x_v[...], (8, D))

        def make_q(slot):
            wq_all(slot).wait()
            if not compute:
                return jnp.zeros((8, GD), jnp.bfloat16)
            qg = jnp.dot(x8, wq_v[slot], preferred_element_type=jnp.float32)
            return jnp.where(diag, qg, 0.0).astype(jnp.bfloat16)

        q0 = make_q(0)
        acc_s[...] = jnp.zeros_like(acc_s)

        def group(g, q, last):
            slot = g % 2
            if last:
                pieces = ffn_pieces(g) + wo_pieces(g)
            else:
                pieces = wq_pieces(g + 1) + ffn_pieces(g) + wo_pieces(g)
            nsteps = 2 * NC
            lim = nsteps - 6
            sched = [[] for _ in range(nsteps)]
            for i, p in enumerate(pieces):
                sched[min(i, lim - 1) if len(pieces) <= lim else (i * lim) // len(pieces)].append(p)

            def tick(step):
                ph, j = divmod(step, NC)
                kv_copy(kt_hbm, g, j).wait()
                for p in sched[step]:
                    p().start(priority=0)
                nxt = step + D1
                if nxt < NC:
                    kv_copy(kt_hbm, g, nxt).start(priority=1)
                elif nxt < 2 * NC:
                    kv_copy(vt_hbm, g, nxt - NC).start(priority=1)
                elif not last:
                    kv_copy(kt_hbm, g + 1, nxt - 2 * NC).start(priority=1)

            ss = []
            for j in range(NC):
                tick(j)
                if compute:
                    ss.append(jnp.dot(q, ring[j], preferred_element_type=jnp.float32))
            if compute:
                m = ss[0]
                for s in ss[1:]:
                    m = jnp.maximum(m, s)
                m = jnp.max(m, axis=-1, keepdims=True)
                ps = [jnp.exp((s - m) * scale) for s in ss]
                l = ps[0]
                for p in ps[1:]:
                    l = l + p
                l = jnp.sum(l, axis=-1, keepdims=True)
                ps = [p.astype(jnp.bfloat16) for p in ps]
            o = jnp.zeros((8, GD), jnp.float32)
            b_scaled = gate = None
            qn = q
            for j in range(NC):
                tick(NC + j)
                if compute:
                    o = o + lax.dot_general(ps[j], ring[j], (((1,), (1,)), ((), ())),
                                            preferred_element_type=jnp.float32)
                if j == 8 and not last:
                    qn = make_q(1 - slot)
                if j == 8 and last:
                    gate, b_scaled = ffn()
            wo_all(slot).wait()
            if compute:
                on = jnp.where(diag, o / l, 0.0).astype(jnp.bfloat16)
                contrib = jnp.dot(on, wo_v[slot], preferred_element_type=jnp.float32)
            else:
                contrib = jnp.zeros((8, D), jnp.float32)
            if last:
                return acc_s[...] + contrib, gate, b_scaled
            acc_s[...] += contrib
            return qn

        def ffn():
            cr.wait(); cg.wait()
            for k, v in enumerate((wg_v, wu_v, wd_v)):
                pltpu.make_async_copy(v, v, fsem.at[k]).wait()
            xf = x_v[...].astype(jnp.float32)
            if not compute:
                return jnp.zeros((1, 1), jnp.float32), xf
            wr = wr_v[...].astype(jnp.float32)
            gw = gw_v[...].astype(jnp.float32)
            r_acc = jnp.zeros((1, 128), jnp.float32)
            g_acc = jnp.zeros((1, 128), jnp.float32)
            for j in range(D // 128):
                xs = xf[:, j * 128:(j + 1) * 128]
                r_acc = r_acc + xs * wr[j:j + 1, :]
                g_acc = g_acc + xs * gw[j:j + 1, :]
            r_sel = jax.nn.sigmoid(jnp.sum(r_acc, axis=-1, keepdims=True))
            gate = jax.nn.sigmoid(jnp.sum(g_acc, axis=-1, keepdims=True))
            gg = jnp.dot(x8, wg_v[...], preferred_element_type=jnp.float32)
            uu = jnp.dot(x8, wu_v[...], preferred_element_type=jnp.float32)
            hh = (gg * jax.nn.sigmoid(gg) * uu).astype(jnp.bfloat16)
            y = jnp.dot(hh, wd_v[...], preferred_element_type=jnp.float32)[0:1, :]
            b = xf + (xf * 0.0 + y * r_sel)
            return gate, (1.0 - gate) * b

        qlast = lax.fori_loop(0, NG - 1, lambda g, q: group(g, q, False), q0)
        acc, gate, b_scaled = group(NG - 1, qlast, True)
        a = jnp.sum(acc, axis=0, keepdims=True)
        out_ref[...] = (gate * a + b_scaled).astype(out_ref.dtype)

    @jax.jit
    def pallas_gated_mix__sliding_block_cached__moe_arch_mod__decode_kernel(A_x, A_k_cache, A_v_cache, A_wq, A_wo, B_x, B_w_r, B_w_gate, B_w_up, B_w_down, gate_w):
        SK = A_k_cache.shape[2]
        W = min(4096, max(256, SK // 4))
        NC = W // CW
        kt = jnp.swapaxes(A_k_cache, 2, 3).reshape(NG, GD, SK)
        vt = jnp.swapaxes(A_v_cache, 2, 3).reshape(NG, GD, SK)
        x = A_x.reshape(1, D)
        wr = B_w_r.reshape(D // 128, 128)
        gw = gate_w.reshape(D // 128, 128)
        bf = jnp.bfloat16
        out = pl.pallas_call(
            kernel,
            out_shape=jax.ShapeDtypeStruct((1, D), bf),
            in_specs=[pl.BlockSpec(memory_space=pl.ANY)] * 10,
            out_specs=pl.BlockSpec(memory_space=pltpu.VMEM),
            scratch_shapes=[
                pltpu.VMEM((1, D), bf), pltpu.VMEM((D // 128, 128), bf), pltpu.VMEM((D // 128, 128), bf),
                pltpu.VMEM((NC, GD, CW), bf),
                pltpu.VMEM((2, D, GD), bf), pltpu.VMEM((2, GD, D), bf),
                pltpu.VMEM((D, F), bf), pltpu.VMEM((D, F), bf), pltpu.VMEM((F, D), bf),
                pltpu.VMEM((8, D), jnp.float32),
                pltpu.SemaphoreType.DMA((3,)), pltpu.SemaphoreType.DMA((NC,)),
                pltpu.SemaphoreType.DMA((2,)), pltpu.SemaphoreType.DMA((2,)), pltpu.SemaphoreType.DMA((3,)),
            ],
            compiler_params=pltpu.CompilerParams(vmem_limit_bytes=64 * 1024 * 1024, disable_bounds_checks=nobc),
        )(x, wr, gw, kt, vt, A_wq, A_wo, B_w_gate, B_w_up, B_w_down)
        return out.reshape(1, 1, D)
    return pallas_gated_mix__sliding_block_cached__moe_arch_mod__decode_kernel


pallas_gated_mix__sliding_block_cached__moe_arch_mod__decode_kernel = _build(wo_piece='col')
```

```python
import functools
import jax
import jax.numpy as jnp
from jax import lax
from jax.experimental import pallas as pl
from jax.experimental.pallas import tpu as pltpu

D = 640
H = 32
DH = 192
F = 1536
G = 2
NG = H // G
GD = G * DH
CW = 128


def _build(D1=16, compute=True, KB=2, VB=2, FJ=8, QJ=8, LIM=6, wo_piece="row16", nobc=True, peel=True):
    def kernel(x_hbm, wr_hbm, gw_hbm, kt_hbm, vt_hbm, wq_hbm, wo_hbm, wg_hbm, wu_hbm, wd_hbm,
               out_ref,
               x_v, wr_v, gw_v, ring, wq_v, wo_v, wg_v, wu_v, wd_v, acc_s,
               ssem, rsem, qsem, osem, fsem):
        SK = kt_hbm.shape[-1]
        NC = ring.shape[0]
        W = NC * CW
        base = SK - W

        def kv_copy(src, g, j):
            return pltpu.make_async_copy(src.at[g, :, pl.ds(base + j * CW, CW)], ring.at[j], rsem.at[j])

        def mo(v, m):
            return v if isinstance(v, int) else pl.multiple_of(v, m)

        def wq_pieces(g):
            slot = g % 2
            out = []
            for c in range(3):
                for r in range(8):
                    out.append(lambda c=c, r=r: pltpu.make_async_copy(
                        wq_hbm.at[pl.ds(r * 80, 80), pl.ds(mo(g * GD + c * 128, 128), 128)],
                        wq_v.at[slot, pl.ds(r * 80, 80), pl.ds(c * 128, 128)], qsem.at[slot]))
            return out

        def wo_pieces(g):
            slot = g % 2
            out = []
            if wo_piece == "row16":
                for i in range(24):
                    out.append(lambda i=i: pltpu.make_async_copy(
                        wo_hbm.at[pl.ds(mo(g * GD + i * 16, 16), 16), :],
                        wo_v.at[slot, pl.ds(i * 16, 16), :], osem.at[slot]))
            else:
                for c in range(5):
                    for r in range(4):
                        out.append(lambda c=c, r=r: pltpu.make_async_copy(
                            wo_hbm.at[pl.ds(mo(g * GD + r * 96, 16), 96), pl.ds(c * 128, 128)],
                            wo_v.at[slot, pl.ds(r * 96, 96), pl.ds(c * 128, 128)], osem.at[slot]))
            return out

        def ffn_pieces(g):
            out = []
            for (src, dst, k) in ((wg_hbm, wg_v, 0), (wu_hbm, wu_v, 1)):
                for i in range(6):
                    def mk(src=src, dst=dst, k=k, i=i):
                        t = g * 6 + i
                        r = mo((t & 7) * 80, 16)
                        c = mo((t >> 3) * 128, 128)
                        return pltpu.make_async_copy(src.at[pl.ds(r, 80), pl.ds(c, 128)],
                                                     dst.at[pl.ds(r, 80), pl.ds(c, 128)], fsem.at[k])
                    out.append(mk)
            for i in range(6):
                def mk(i=i):
                    if wo_piece == "row16":
                        r = mo(g * 96 + i * 16, 16)
                        return pltpu.make_async_copy(wd_hbm.at[pl.ds(r, 16), :], wd_v.at[pl.ds(r, 16), :], fsem.at[2])
                    else:
                        if i == 5:
                            return None
                        r = mo(g * 96, 16)
                        return pltpu.make_async_copy(wd_hbm.at[pl.ds(r, 96), pl.ds(i * 128, 128)],
                                                     wd_v.at[pl.ds(r, 96), pl.ds(i * 128, 128)], fsem.at[2])
                out.append(mk)
            if wo_piece != "row16":
                out = out[:-1]
            return out

        cx = pltpu.make_async_copy(x_hbm, x_v, ssem.at[0])
        cr = pltpu.make_async_copy(wr_hbm, wr_v, ssem.at[1])
        cg = pltpu.make_async_copy(gw_hbm, gw_v, ssem.at[2])

        def wq_all(slot):
            return pltpu.make_async_copy(wq_v.at[slot], wq_v.at[slot], qsem.at[slot])

        def wo_all(slot):
            return pltpu.make_async_copy(wo_v.at[slot], wo_v.at[slot], osem.at[slot])

        kv_copy(kt_hbm, 0, 0).start(priority=1)
        pltpu.make_async_copy(wq_hbm.at[:, pl.ds(0, GD)], wq_v.at[0], qsem.at[0]).start(priority=0)
        cx.start()
        for j in range(1, D1):
            kv_copy(kt_hbm, 0, j).start(priority=1)
        cr.start(); cg.start()

        row = lax.broadcasted_iota(jnp.int32, (8, GD), 0)
        col = lax.broadcasted_iota(jnp.int32, (8, GD), 1)
        diag = (col >= row * DH) & (col < (row + 1) * DH)
        scale = DH ** -0.5

        cx.wait()
        x8 = jnp.broadcast_to(x_v[...], (8, D))

        def make_q(slot):
            wq_all(slot).wait()
            if not compute:
                return jnp.zeros((8, GD), jnp.bfloat16)
            qg = jnp.dot(x8, wq_v[slot], preferred_element_type=jnp.float32)
            return jnp.where(diag, qg, 0.0).astype(jnp.bfloat16)

        q0 = make_q(0)
        acc_s[...] = jnp.zeros_like(acc_s)

        def group(g, q, last):
            slot = g % 2
            if last:
                pieces = ffn_pieces(g) + wo_pieces(g)
            else:
                pieces = wq_pieces(g + 1) + ffn_pieces(g) + wo_pieces(g)
            nsteps = 2 * NC
            lim = nsteps - LIM
            sched = [[] for _ in range(nsteps)]
            for i, p in enumerate(pieces):
                sched[min(i, lim - 1) if len(pieces) <= lim else (i * lim) // len(pieces)].append(p)

            def tick(step):
                ph, j = divmod(step, NC)
                kv_copy(kt_hbm, g, j).wait()
                for p in sched[step]:
                    p().start(priority=0)
                nxt = step + D1
                if nxt < NC:
                    kv_copy(kt_hbm, g, nxt).start(priority=1)
                elif nxt < 2 * NC:
                    kv_copy(vt_hbm, g, nxt - NC).start(priority=1)
                elif not last:
                    kv_copy(kt_hbm, g + 1, nxt - 2 * NC).start(priority=1)

            ss = []
            for j in range(NC):
                tick(j)
                if compute and (j + 1) % KB == 0:
                    for jj in range(j + 1 - KB, j + 1):
                        ss.append(jnp.dot(q, ring[jj], preferred_element_type=jnp.float32))
            if compute:
                m = ss[0]
                for s in ss[1:]:
                    m = jnp.maximum(m, s)
                m = jnp.max(m, axis=-1, keepdims=True)
                ps = [jnp.exp((s - m) * scale) for s in ss]
                l = ps[0]
                for p in ps[1:]:
                    l = l + p
                l = jnp.sum(l, axis=-1, keepdims=True)
                ps = [p.astype(jnp.bfloat16) for p in ps]
            o = jnp.zeros((8, GD), jnp.float32)
            b_scaled = gate = None
            qn = q
            for j in range(NC):
                tick(NC + j)
                if compute and (j + 1) % VB == 0:
                    for jj in range(j + 1 - VB, j + 1):
                        o = o + lax.dot_general(ps[jj], ring[jj], (((1,), (1,)), ((), ())),
                                                preferred_element_type=jnp.float32)
                if j == QJ and not last:
                    qn = make_q(1 - slot)
                if j == FJ and last:
                    gate, b_scaled = ffn()
            wo_all(slot).wait()
            if compute:
                on = jnp.where(diag, o / l, 0.0).astype(jnp.bfloat16)
                contrib = jnp.dot(on, wo_v[slot], preferred_element_type=jnp.float32)
            else:
                contrib = jnp.zeros((8, D), jnp.float32)
            if last:
                return acc_s[...] + contrib, gate, b_scaled
            acc_s[...] += contrib
            return qn

        def ffn():
            cr.wait(); cg.wait()
            for k, v in enumerate((wg_v, wu_v, wd_v)):
                pltpu.make_async_copy(v, v, fsem.at[k]).wait()
            xf = x_v[...].astype(jnp.float32)
            if not compute:
                return jnp.zeros((1, 1), jnp.float32), xf
            wr = wr_v[...].astype(jnp.float32)
            gw = gw_v[...].astype(jnp.float32)
            r_acc = jnp.zeros((1, 128), jnp.float32)
            g_acc = jnp.zeros((1, 128), jnp.float32)
            for j in range(D // 128):
                xs = xf[:, j * 128:(j + 1) * 128]
                r_acc = r_acc + xs * wr[j:j + 1, :]
                g_acc = g_acc + xs * gw[j:j + 1, :]
            r_sel = jax.nn.sigmoid(jnp.sum(r_acc, axis=-1, keepdims=True))
            gate = jax.nn.sigmoid(jnp.sum(g_acc, axis=-1, keepdims=True))
            gg = jnp.dot(x8, wg_v[...], preferred_element_type=jnp.float32)
            uu = jnp.dot(x8, wu_v[...], preferred_element_type=jnp.float32)
            hh = (gg * jax.nn.sigmoid(gg) * uu).astype(jnp.bfloat16)
            y = jnp.dot(hh, wd_v[...], preferred_element_type=jnp.float32)[0:1, :]
            b = xf + (xf * 0.0 + y * r_sel)
            return gate, (1.0 - gate) * b

        qlast = lax.fori_loop(0, NG - 1, lambda g, q: group(g, q, False), q0)
        acc, gate, b_scaled = group(NG - 1, qlast, True)
        a = jnp.sum(acc, axis=0, keepdims=True)
        out_ref[...] = (gate * a + b_scaled).astype(out_ref.dtype)

    @jax.jit
    def pallas_gated_mix__sliding_block_cached__moe_arch_mod__decode_kernel(A_x, A_k_cache, A_v_cache, A_wq, A_wo, B_x, B_w_r, B_w_gate, B_w_up, B_w_down, gate_w):
        SK = A_k_cache.shape[2]
        W = min(4096, max(256, SK // 4))
        NC = W // CW
        kt = jnp.swapaxes(A_k_cache, 2, 3).reshape(NG, GD, SK)
        vt = jnp.swapaxes(A_v_cache, 2, 3).reshape(NG, GD, SK)
        x = A_x.reshape(1, D)
        wr = B_w_r.reshape(D // 128, 128)
        gw = gate_w.reshape(D // 128, 128)
        bf = jnp.bfloat16
        out = pl.pallas_call(
            kernel,
            out_shape=jax.ShapeDtypeStruct((1, D), bf),
            in_specs=[pl.BlockSpec(memory_space=pl.ANY)] * 10,
            out_specs=pl.BlockSpec(memory_space=pltpu.VMEM),
            scratch_shapes=[
                pltpu.VMEM((1, D), bf), pltpu.VMEM((D // 128, 128), bf), pltpu.VMEM((D // 128, 128), bf),
                pltpu.VMEM((NC, GD, CW), bf),
                pltpu.VMEM((2, D, GD), bf), pltpu.VMEM((2, GD, D), bf),
                pltpu.VMEM((D, F), bf), pltpu.VMEM((D, F), bf), pltpu.VMEM((F, D), bf),
                pltpu.VMEM((8, D), jnp.float32),
                pltpu.SemaphoreType.DMA((3,)), pltpu.SemaphoreType.DMA((NC,)),
                pltpu.SemaphoreType.DMA((2,)), pltpu.SemaphoreType.DMA((2,)), pltpu.SemaphoreType.DMA((3,)),
            ],
            compiler_params=pltpu.CompilerParams(vmem_limit_bytes=64 * 1024 * 1024, disable_bounds_checks=nobc),
        )(x, wr, gw, kt, vt, A_wq, A_wo, B_w_gate, B_w_up, B_w_down)
        return out.reshape(1, 1, D)
    return pallas_gated_mix__sliding_block_cached__moe_arch_mod__decode_kernel


pallas_gated_mix__sliding_block_cached__moe_arch_mod__decode_kernel = _build(wo_piece='col',KB=2,VB=2,LIM=3,FJ=1,QJ=1)
```

```python
import functools
import jax
import jax.numpy as jnp
from jax import lax
from jax.experimental import pallas as pl
from jax.experimental.pallas import tpu as pltpu

D = 640
H = 32
DH = 192
F = 1536
G = 2
NG = H // G
GD = G * DH
CW = 128


def _build(D1=16, compute=True, KB=2, VB=2, FJ=8, QJ=8, LIM=6, wo_piece="row16", nobc=True, peel=True):
    def kernel(x_hbm, wr_hbm, gw_hbm, kt_hbm, vt_hbm, wq_hbm, wo_hbm, wg_hbm, wu_hbm, wd_hbm,
               out_ref,
               x_v, wr_v, gw_v, ring, wq_v, wo_v, wg_v, wu_v, wd_v, acc_s):
        dma = pltpu.SemaphoreType.DMA
        pl.run_scoped(
            functools.partial(body, x_hbm, wr_hbm, gw_hbm, kt_hbm, vt_hbm, wq_hbm, wo_hbm, wg_hbm, wu_hbm, wd_hbm,
                              out_ref, x_v, wr_v, gw_v, ring, wq_v, wo_v, wg_v, wu_v, wd_v, acc_s),
            dma((3,)), dma((ring.shape[0],)), dma((2,)), dma((2,)), dma((3,)))

    def body(x_hbm, wr_hbm, gw_hbm, kt_hbm, vt_hbm, wq_hbm, wo_hbm, wg_hbm, wu_hbm, wd_hbm,
             out_ref,
             x_v, wr_v, gw_v, ring, wq_v, wo_v, wg_v, wu_v, wd_v, acc_s,
             ssem, rsem, qsem, osem, fsem):
        SK = kt_hbm.shape[-1]
        NC = ring.shape[0]
        W = NC * CW
        base = SK - W

        def kv_copy(src, g, j):
            return pltpu.make_async_copy(src.at[g, :, pl.ds(base + j * CW, CW)], ring.at[j], rsem.at[j])

        def mo(v, m):
            return v if isinstance(v, int) else pl.multiple_of(v, m)

        def wq_pieces(g):
            slot = g % 2
            out = []
            for c in range(3):
                for r in range(8):
                    out.append(lambda c=c, r=r: pltpu.make_async_copy(
                        wq_hbm.at[pl.ds(r * 80, 80), pl.ds(mo(g * GD + c * 128, 128), 128)],
                        wq_v.at[slot, pl.ds(r * 80, 80), pl.ds(c * 128, 128)], qsem.at[slot]))
            return out

        def wo_pieces(g):
            slot = g % 2
            out = []
            if wo_piece == "row16":
                for i in range(24):
                    out.append(lambda i=i: pltpu.make_async_copy(
                        wo_hbm.at[pl.ds(mo(g * GD + i * 16, 16), 16), :],
                        wo_v.at[slot, pl.ds(i * 16, 16), :], osem.at[slot]))
            else:
                for c in range(5):
                    for r in range(4):
                        out.append(lambda c=c, r=r: pltpu.make_async_copy(
                            wo_hbm.at[pl.ds(mo(g * GD + r * 96, 16), 96), pl.ds(c * 128, 128)],
                            wo_v.at[slot, pl.ds(r * 96, 96), pl.ds(c * 128, 128)], osem.at[slot]))
            return out

        def ffn_pieces(g):
            out = []
            for (src, dst, k) in ((wg_hbm, wg_v, 0), (wu_hbm, wu_v, 1)):
                for i in range(6):
                    def mk(src=src, dst=dst, k=k, i=i):
                        t = g * 6 + i
                        r = mo((t & 7) * 80, 16)
                        c = mo((t >> 3) * 128, 128)
                        return pltpu.make_async_copy(src.at[pl.ds(r, 80), pl.ds(c, 128)],
                                                     dst.at[pl.ds(r, 80), pl.ds(c, 128)], fsem.at[k])
                    out.append(mk)
            for i in range(6):
                def mk(i=i):
                    if wo_piece == "row16":
                        r = mo(g * 96 + i * 16, 16)
                        return pltpu.make_async_copy(wd_hbm.at[pl.ds(r, 16), :], wd_v.at[pl.ds(r, 16), :], fsem.at[2])
                    else:
                        if i == 5:
                            return None
                        r = mo(g * 96, 16)
                        return pltpu.make_async_copy(wd_hbm.at[pl.ds(r, 96), pl.ds(i * 128, 128)],
                                                     wd_v.at[pl.ds(r, 96), pl.ds(i * 128, 128)], fsem.at[2])
                out.append(mk)
            if wo_piece != "row16":
                out = out[:-1]
            return out

        cx = pltpu.make_async_copy(x_hbm, x_v, ssem.at[0])
        cr = pltpu.make_async_copy(wr_hbm, wr_v, ssem.at[1])
        cg = pltpu.make_async_copy(gw_hbm, gw_v, ssem.at[2])

        def wq_all(slot):
            return pltpu.make_async_copy(wq_v.at[slot], wq_v.at[slot], qsem.at[slot])

        def wo_all(slot):
            return pltpu.make_async_copy(wo_v.at[slot], wo_v.at[slot], osem.at[slot])

        kv_copy(kt_hbm, 0, 0).start(priority=1)
        pltpu.make_async_copy(wq_hbm.at[:, pl.ds(0, GD)], wq_v.at[0], qsem.at[0]).start(priority=0)
        cx.start()
        for j in range(1, D1):
            kv_copy(kt_hbm, 0, j).start(priority=1)
        cr.start(); cg.start()

        row = lax.broadcasted_iota(jnp.int32, (8, GD), 0)
        col = lax.broadcasted_iota(jnp.int32, (8, GD), 1)
        diag = (col >= row * DH) & (col < (row + 1) * DH)
        scale = DH ** -0.5

        cx.wait()
        x8 = jnp.broadcast_to(x_v[...], (8, D))

        def make_q(slot):
            wq_all(slot).wait()
            if not compute:
                return jnp.zeros((8, GD), jnp.bfloat16)
            qg = jnp.dot(x8, wq_v[slot], preferred_element_type=jnp.float32)
            return jnp.where(diag, qg, 0.0).astype(jnp.bfloat16)

        q0 = make_q(0)
        acc_s[...] = jnp.zeros_like(acc_s)

        def group(g, q, last):
            slot = g % 2
            if last:
                pieces = ffn_pieces(g) + wo_pieces(g)
            else:
                pieces = wq_pieces(g + 1) + ffn_pieces(g) + wo_pieces(g)
            nsteps = 2 * NC
            lim = nsteps - LIM
            sched = [[] for _ in range(nsteps)]
            for i, p in enumerate(pieces):
                sched[min(i, lim - 1) if len(pieces) <= lim else (i * lim) // len(pieces)].append(p)

            def tick(step):
                ph, j = divmod(step, NC)
                kv_copy(kt_hbm, g, j).wait()
                for p in sched[step]:
                    p().start(priority=0)
                nxt = step + D1
                if nxt < NC:
                    kv_copy(kt_hbm, g, nxt).start(priority=1)
                elif nxt < 2 * NC:
                    kv_copy(vt_hbm, g, nxt - NC).start(priority=1)
                elif not last:
                    kv_copy(kt_hbm, g + 1, nxt - 2 * NC).start(priority=1)

            ss = []
            for j in range(NC):
                tick(j)
                if compute and (j + 1) % KB == 0:
                    for jj in range(j + 1 - KB, j + 1):
                        ss.append(jnp.dot(q, ring[jj], preferred_element_type=jnp.float32))
            if compute:
                m = ss[0]
                for s in ss[1:]:
                    m = jnp.maximum(m, s)
                m = jnp.max(m, axis=-1, keepdims=True)
                ps = [jnp.exp((s - m) * scale) for s in ss]
                l = ps[0]
                for p in ps[1:]:
                    l = l + p
                l = jnp.sum(l, axis=-1, keepdims=True)
                ps = [p.astype(jnp.bfloat16) for p in ps]
            o = jnp.zeros((8, GD), jnp.float32)
            b_scaled = gate = None
            qn = q
            for j in range(NC):
                tick(NC + j)
                if compute and (j + 1) % VB == 0:
                    for jj in range(j + 1 - VB, j + 1):
                        o = o + lax.dot_general(ps[jj], ring[jj], (((1,), (1,)), ((), ())),
                                                preferred_element_type=jnp.float32)
                if j == QJ and not last:
                    qn = make_q(1 - slot)
                if j == FJ and last:
                    gate, b_scaled = ffn()
            wo_all(slot).wait()
            if compute:
                on = jnp.where(diag, o / l, 0.0).astype(jnp.bfloat16)
                contrib = jnp.dot(on, wo_v[slot], preferred_element_type=jnp.float32)
            else:
                contrib = jnp.zeros((8, D), jnp.float32)
            if last:
                return acc_s[...] + contrib, gate, b_scaled
            acc_s[...] += contrib
            return qn

        def ffn():
            cr.wait(); cg.wait()
            for k, v in enumerate((wg_v, wu_v, wd_v)):
                pltpu.make_async_copy(v, v, fsem.at[k]).wait()
            xf = x_v[...].astype(jnp.float32)
            if not compute:
                return jnp.zeros((1, 1), jnp.float32), xf
            wr = wr_v[...].astype(jnp.float32)
            gw = gw_v[...].astype(jnp.float32)
            r_acc = jnp.zeros((1, 128), jnp.float32)
            g_acc = jnp.zeros((1, 128), jnp.float32)
            for j in range(D // 128):
                xs = xf[:, j * 128:(j + 1) * 128]
                r_acc = r_acc + xs * wr[j:j + 1, :]
                g_acc = g_acc + xs * gw[j:j + 1, :]
            r_sel = jax.nn.sigmoid(jnp.sum(r_acc, axis=-1, keepdims=True))
            gate = jax.nn.sigmoid(jnp.sum(g_acc, axis=-1, keepdims=True))
            gg = jnp.dot(x8, wg_v[...], preferred_element_type=jnp.float32)
            uu = jnp.dot(x8, wu_v[...], preferred_element_type=jnp.float32)
            hh = (gg * jax.nn.sigmoid(gg) * uu).astype(jnp.bfloat16)
            y = jnp.dot(hh, wd_v[...], preferred_element_type=jnp.float32)[0:1, :]
            b = xf + (xf * 0.0 + y * r_sel)
            return gate, (1.0 - gate) * b

        qlast = lax.fori_loop(0, NG - 1, lambda g, q: group(g, q, False), q0)
        acc, gate, b_scaled = group(NG - 1, qlast, True)
        a = jnp.sum(acc, axis=0, keepdims=True)
        out_ref[...] = (gate * a + b_scaled).astype(out_ref.dtype)

    @jax.jit
    def pallas_gated_mix__sliding_block_cached__moe_arch_mod__decode_kernel(A_x, A_k_cache, A_v_cache, A_wq, A_wo, B_x, B_w_r, B_w_gate, B_w_up, B_w_down, gate_w):
        SK = A_k_cache.shape[2]
        W = min(4096, max(256, SK // 4))
        NC = W // CW
        kt = jnp.swapaxes(A_k_cache, 2, 3).reshape(NG, GD, SK)
        vt = jnp.swapaxes(A_v_cache, 2, 3).reshape(NG, GD, SK)
        x = A_x.reshape(1, D)
        wr = B_w_r.reshape(D // 128, 128)
        gw = gate_w.reshape(D // 128, 128)
        bf = jnp.bfloat16
        out = pl.pallas_call(
            kernel,
            out_shape=jax.ShapeDtypeStruct((1, D), bf),
            in_specs=[pl.BlockSpec(memory_space=pl.ANY)] * 10,
            out_specs=pl.BlockSpec(memory_space=pltpu.VMEM),
            scratch_shapes=[
                pltpu.VMEM((1, D), bf), pltpu.VMEM((D // 128, 128), bf), pltpu.VMEM((D // 128, 128), bf),
                pltpu.VMEM((NC, GD, CW), bf),
                pltpu.VMEM((2, D, GD), bf), pltpu.VMEM((2, GD, D), bf),
                pltpu.VMEM((D, F), bf), pltpu.VMEM((D, F), bf), pltpu.VMEM((F, D), bf),
                pltpu.VMEM((8, D), jnp.float32),
            ],
            compiler_params=pltpu.CompilerParams(vmem_limit_bytes=64 * 1024 * 1024, disable_bounds_checks=nobc),
        )(x, wr, gw, kt, vt, A_wq, A_wo, B_w_gate, B_w_up, B_w_down)
        return out.reshape(1, 1, D)
    return pallas_gated_mix__sliding_block_cached__moe_arch_mod__decode_kernel


pallas_gated_mix__sliding_block_cached__moe_arch_mod__decode_kernel = _build(wo_piece='col',KB=2,VB=2,LIM=3,FJ=1,QJ=1)
```

```python
import functools
import jax
import jax.numpy as jnp
from jax import lax
from jax.experimental import pallas as pl
from jax.experimental.pallas import tpu as pltpu

D = 640
H = 32
DH = 192
F = 1536
G = 4
NG = H // G
GD = G * DH
CW = 128
NT = GD // 128


def _build(D1=15, RU=8, SR=256, compute=True, use=(0, 1, 2, 3), pq=(40, 128), po=(8, 640), pf=(8, 768), pd=(8, 640), FR=88, AL=8, rowmajor_o=True,
          n2=32, LAG=2, pin=False, lastlim=0, nobc=True):
    NS = GD // SR
    FR0 = D - (NG - 1) * FR
    bf16 = jnp.bfloat16
    f32 = jnp.float32

    def kernel(*refs):
        dma = pltpu.SemaphoreType.DMA
        pl.run_scoped(functools.partial(body, *refs),
                      dma((3,)), dma((RU * NS,)), dma((1,)), dma((2,)), dma((2,)), dma((F // 128,)))

    def body(x_hbm, wr_hbm, gw_hbm, kt_hbm, vt_hbm, wq_hbm, wo_hbm, wg_hbm, wu_hbm, wd_hbm,
             out_ref,
             x_v, wr_v, gw_v, ring, wq_v, wo_v, wg_v, wu_v, wd_v, acc_s,
             ssem, rsem, qsem, osem, fsem, dsem):
        SK = kt_hbm.shape[-1]
        W = min(4096, max(256, SK // 4))
        NC = W // CW
        base = SK - W

        def mo(v, m):
            return v if isinstance(v, int) else pl.multiple_of(v, m)

        def p1(g, i):
            u, s = divmod(i, NS)
            rows = pl.ds(s * SR, SR)
            if u < NC:
                src = kt_hbm.at[g, rows, pl.ds(base + u * CW, CW)]
            elif u < 2 * NC:
                src = vt_hbm.at[g, rows, pl.ds(base + (u - NC) * CW, CW)]
            else:
                src = wo_hbm.at[pl.ds(g * GD + s * SR, SR), pl.ds((u - 2 * NC) * CW, CW)]
            return pltpu.make_async_copy(src, ring.at[u % RU, rows, :], rsem.at[(u % RU) * NS + s])

        def rect(src, dst, r0, nr, c0, nc, dr0, dc0, shp, sem):
            out = []
            pr, pc = shp
            for c in range(0, nc, pc):
                for r in range(0, nr, pr):
                    h = min(pr, nr - r)
                    w = min(pc, nc - c)

                    def mk(r=r, c=c, h=h, w=w):
                        d = dst.at[pl.ds(mo(dr0 + r, AL), h), pl.ds(mo(dc0 + c, 128), w)]
                        return pltpu.make_async_copy(
                            src.at[pl.ds(mo(r0 + r, AL), h), pl.ds(mo(c0 + c, 128), w)], d, sem), d
                    out.append(mk)
            return out

        def rect_rows(src, dst, r0, nr, nc, shp, sem, dr0=None):
            out = []
            for r in range(0, nr, shp[0]):
                out += rect(src, dst, r0 + r, min(shp[0], nr - r), 0, nc, (r0 if dr0 is None else dr0) + r, 0, shp, sem)
            return out

        def wq_pieces(g):
            return rect(wq_hbm, wq_v, 0, D, g * GD, GD, 0, 0, pq, qsem.at[0])

        def wo_pieces(g):
            return rect_rows(wo_hbm, wo_v.at[g % 2], g * GD, GD, D, po, osem.at[g % 2], dr0=0)

        def gu_pieces(r0, nr):
            a = rect_rows(wg_hbm, wg_v, r0, nr, F, pf, fsem.at[0])
            b = rect_rows(wu_hbm, wu_v, r0, nr, F, pf, fsem.at[1])
            return [p for ab in zip(a, b) for p in ab]

        def wd_pieces():
            out = []
            for b in range(F // 128):
                out += rect_rows(wd_hbm, wd_v, b * 128, 128, D, pd, dsem.at[b])
            return out

        def wait_full(ref, sem):
            pltpu.make_async_copy(ref, ref, sem).wait()

        cx = pltpu.make_async_copy(x_hbm, x_v, ssem.at[0])
        cr = pltpu.make_async_copy(wr_hbm, wr_v, ssem.at[1])
        cg = pltpu.make_async_copy(gw_hbm, gw_v, ssem.at[2])

        p1(0, 0).start(priority=1)
        pltpu.make_async_copy(wq_hbm.at[:, pl.ds(0, GD)], wq_v, qsem.at[0]).start(priority=0)
        cx.start()
        for i in range(1, D1):
            p1(0, i).start(priority=1)
        cr.start(); cg.start()

        row = lax.broadcasted_iota(jnp.int32, (8, GD), 0)
        col = lax.broadcasted_iota(jnp.int32, (8, GD), 1)
        diag = (col >= row * DH) & (col < (row + 1) * DH)
        scale = DH ** -0.5

        acc_s[...] = jnp.zeros_like(acc_s)
        wo_v[1] = jnp.zeros((GD, D), bf16)
        cx.wait()
        x8 = jnp.broadcast_to(x_v[...], (8, D))

        def q_tile(t):
            if not compute:
                return jnp.zeros((8, 128), bf16)
            qt = jnp.dot(x8, wq_v[:, t * 128:(t + 1) * 128], preferred_element_type=f32)
            return jnp.where(diag[:, t * 128:(t + 1) * 128], qt, 0.0).astype(bf16)

        wait_full(wq_v, qsem.at[0])
        q0 = jnp.concatenate([q_tile(t) for t in range(NT)], axis=1)

        def assign(pieces_at, nunits):
            slots = [(u, k) for u in range(nunits) for k in use]
            sched = {}
            for lo, hi, ps in pieces_at:
                n = hi - lo
                for i, p in enumerate(ps):
                    sched.setdefault(slots[lo + (i * n) // len(ps)], []).append(p)
            return sched

        def group(g, q, on_prev, last):
            nunits = 2 * NC + (D // CW if last else 0)
            L = nunits * NS
            nsl = 2 * NC * len(use)
            if last:
                gu = gu_pieces(0, FR0)
                wd = wd_pieces()
                n1 = (len(gu) * (nsl - lastlim)) // (len(gu) + len(wd))
                sched = assign([(0, n1, gu), (n1, nsl - lastlim, wd)], nunits)
                wd_unit = {}
                per = len(wd) // (F // 128)
                for (u, k), ps in sched.items():
                    for p in ps:
                        if p in wd and wd.index(p) % per == per - 1:
                            wd_unit[wd.index(p) // per] = u
                HW = max(D // CW, LAG + max(u for (u, k), ps in sched.items() if any(p in gu for p in ps)))
            else:
                gu = gu_pieces(FR0 + g * FR, FR)
                m2 = min(n2, len(gu))
                wqp = wq_pieces(g + 1)
                wop = wo_pieces(g)
                seq = gu[:len(gu) - m2] + wop + wqp + gu[len(gu) - m2:]
                sched = assign([(0, nsl, seq)], nunits)
                QW = LAG + max(u for (u, k), ps in sched.items() if any(p in wqp for p in ps)) - NC
                assert 0 <= QW < NC
                assert max(u for (u, k), ps in sched.items() if any(p in wop for p in ps)) < 2 * NC - 1

            def issue(u, k, pin_val=None):
                for p in sched.get((u, k), []):
                    cp, dref = p()
                    if pin_val is not None:
                        pv = pin_val if AL == 8 else jnp.concatenate([pin_val, pin_val], axis=0)
                        dref[0:AL, 0:128] = pv.astype(bf16)
                    cp.start(priority=0)

            def ticks(u):
                for s in range(NS):
                    i = u * NS + s
                    p1(g, i).wait()
                    issue(u, s + 3 - NS)
                    nxt = i + D1
                    if nxt < L:
                        p1(g, nxt).start(priority=1)
                    elif not last:
                        p1(g + 1, nxt - L).start(priority=1)

            slot_prev = (g + 1) % 2
            ss = []
            mrun = None
            hs = []
            y = None
            ydone = 0
            stash = {}

            def extras(u):
                nonlocal y, ydone
                if not compute:
                    return
                if u < D // CW:
                    c = u
                    acc_s[:, c * CW:(c + 1) * CW] += jnp.dot(on_prev, wo_v[slot_prev, :, c * CW:(c + 1) * CW],
                                                             preferred_element_type=f32)
                if last:
                    if HW <= u < HW + F // 128:
                        c = u - HW
                        gg = jnp.dot(x8, wg_v[:, c * 128:(c + 1) * 128], preferred_element_type=f32)
                        uu = jnp.dot(x8, wu_v[:, c * 128:(c + 1) * 128], preferred_element_type=f32)
                        hs.append((gg * jax.nn.sigmoid(gg) * uu).astype(bf16))
                    elif stash.get("wd", 0) > ydone and len(hs) > ydone:
                        b = ydone
                        part = jnp.dot(hs[b], wd_v[b * 128:(b + 1) * 128, :], preferred_element_type=f32)
                        y = part if y is None else y + part
                        ydone += 1

            def waits(u):
                if last:
                    if u == HW:
                        wait_full(wg_v, fsem.at[0])
                        wait_full(wu_v, fsem.at[1])
                    b = stash.get("wd", 0)
                    while b < F // 128 and u >= wd_unit[b] + LAG:
                        wait_full(wd_v.at[pl.ds(b * 128, 128), :], dsem.at[b])
                        b += 1
                    stash["wd"] = b
                else:
                    if u == NC + QW:
                        wait_full(wq_v, qsem.at[0])
                    if u == 2 * NC - 1:
                        wait_full(wo_v.at[g % 2], osem.at[g % 2])

            for u in range(NC):
                waits(u)
                ticks(u)
                if compute:
                    kk = ring.at[u % RU]
                    parts = [jnp.dot(q[:, t * 128:(t + 1) * 128], kk[t * 128:(t + 1) * 128, :],
                                     preferred_element_type=f32) for t in range(NT)]
                    issue(u, 3, parts[0] if pin else None)
                    s = parts[0]
                    for pp in parts[1:]:
                        s = s + pp
                    ss.append(s)
                    mrun = s if mrun is None else jnp.maximum(mrun, s)
                else:
                    issue(u, 3)
                extras(u)
            if compute:
                m = jnp.max(mrun, axis=-1, keepdims=True)
            o = [jnp.zeros((8, 128), f32) for _ in range(NT)]
            lrun = jnp.zeros((8, 128), f32)
            qn = []
            for j in range(NC):
                u = NC + j
                waits(u)
                ticks(u)
                if compute:
                    vv = ring.at[u % RU]
                    p = jnp.exp((ss[j] - m) * scale)
                    lrun = lrun + p
                    pb = p.astype(bf16)
                    parts = [lax.dot_general(pb, vv[t * 128:(t + 1) * 128, :], (((1,), (1,)), ((), ())),
                                             preferred_element_type=f32) for t in range(NT)]
                    issue(u, 3, parts[0] if pin else None)
                    o = [a + b for a, b in zip(o, parts)]
                else:
                    issue(u, 3)
                if not last and j >= QW:
                    todo = NT - len(qn)
                    left = NC - j
                    for _ in range(-(-todo // left)):
                        qn.append(q_tile(len(qn)))
                extras(u)
            if compute:
                l = jnp.sum(lrun, axis=-1, keepdims=True)
                on = jnp.where(diag, jnp.concatenate(o, axis=1) / l, 0.0).astype(bf16)
            else:
                on = on_prev
            if not last:
                return jnp.concatenate(qn, axis=1), on

            cr.wait(); cg.wait()
            xf = x_v[...].astype(f32)
            wr = wr_v[...].astype(f32)
            gw = gw_v[...].astype(f32)
            r_acc = jnp.zeros((1, 128), f32)
            g_acc = jnp.zeros((1, 128), f32)
            for j in range(D // 128):
                xs = xf[:, j * 128:(j + 1) * 128]
                r_acc = r_acc + xs * wr[j:j + 1, :]
                g_acc = g_acc + xs * gw[j:j + 1, :]
            r_sel = jax.nn.sigmoid(jnp.sum(r_acc, axis=-1, keepdims=True))
            gate = jax.nn.sigmoid(jnp.sum(g_acc, axis=-1, keepdims=True))
            res = []
            for c in range(D // CW):
                u = 2 * NC + c
                waits(u)
                ticks(u)
                if compute:
                    a = acc_s[:, c * CW:(c + 1) * CW] + jnp.dot(on, ring[u % RU], preferred_element_type=f32)
                    res.append(jnp.sum(a, axis=0, keepdims=True))
                if c < D // CW - 1:
                    while compute and stash["wd"] > ydone:
                        extras(u)
            assert stash["wd"] == F // 128
            if compute:
                assert ydone == F // 128
                b = xf + (xf * 0.0 + y[0:1, :] * r_sel)
                out_ref[...] = (gate * jnp.concatenate(res, axis=1) + (1.0 - gate) * b).astype(out_ref.dtype)
            else:
                out_ref[...] = (gate * xf).astype(out_ref.dtype)

        on0 = jnp.zeros((8, GD), bf16)
        qlast, onlast = lax.fori_loop(0, NG - 1, lambda g, c: group(g, c[0], c[1], False), (q0, on0))
        group(NG - 1, qlast, onlast, True)

    @jax.jit
    def pallas_gated_mix__sliding_block_cached__moe_arch_mod__decode_kernel(A_x, A_k_cache, A_v_cache, A_wq, A_wo, B_x, B_w_r, B_w_gate, B_w_up, B_w_down, gate_w):
        SK = A_k_cache.shape[2]
        kt = jnp.swapaxes(A_k_cache, 2, 3).reshape(NG, GD, SK)
        vt = jnp.swapaxes(A_v_cache, 2, 3).reshape(NG, GD, SK)
        x = A_x.reshape(1, D)
        wr = B_w_r.reshape(D // 128, 128)
        gw = gate_w.reshape(D // 128, 128)
        bf = jnp.bfloat16
        out = pl.pallas_call(
            kernel,
            out_shape=jax.ShapeDtypeStruct((1, D), bf),
            in_specs=[pl.BlockSpec(memory_space=pl.ANY)] * 10,
            out_specs=pl.BlockSpec(memory_space=pltpu.VMEM),
            scratch_shapes=[
                pltpu.VMEM((1, D), bf), pltpu.VMEM((D // 128, 128), bf), pltpu.VMEM((D // 128, 128), bf),
                pltpu.VMEM((RU, GD, CW), bf),
                pltpu.VMEM((D, GD), bf), pltpu.VMEM((2, GD, D), bf),
                pltpu.VMEM((D, F), bf), pltpu.VMEM((D, F), bf), pltpu.VMEM((F, D), bf),
                pltpu.VMEM((8, D), jnp.float32),
            ],
            compiler_params=pltpu.CompilerParams(vmem_limit_bytes=64 * 1024 * 1024, disable_bounds_checks=nobc),
        )(x, wr, gw, kt, vt, A_wq, A_wo, B_w_gate, B_w_up, B_w_down)
        return out.reshape(1, 1, D)
    return pallas_gated_mix__sliding_block_cached__moe_arch_mod__decode_kernel


pallas_gated_mix__sliding_block_cached__moe_arch_mod__decode_kernel = _build(pin=True,AL=16,FR=80,pq=(32,128),po=(16,384),pf=(16,384),pd=(16,384))
```

```python
import contextlib
import functools
import jax
import jax.numpy as jnp
from jax import lax
from jax.experimental import pallas as pl
from jax.experimental.pallas import tpu as pltpu

D = 640
H = 32
DH = 192
F = 1536
G = 4
NG = H // G
GD = G * DH
CW = 128
NT = GD // 128


def _build(D1=15, RU=8, SR=256, compute=True, use=None, mids=(0,), pq=(40, 128), po=(8, 640), pf=(8, 768), pd=(8, 640), FR=88, AL=8, QB=8, pq3=None, qorder='r',
          n2=32, LAG=2, pin=False, lastlim=0, nobc=True, scopes=False, ft=True, goff=0, BW=32):
    NS = GD // SR
    FR0 = D - (NG - 1) * FR
    RS = RU * NS
    TPS = SR // 128
    if use is None:
        use = tuple(range(NS + len(mids)))
    bf16 = jnp.bfloat16
    f32 = jnp.float32
    scope = jax.named_scope if scopes else (lambda name: contextlib.nullcontext())

    def kernel(*refs):
        dma = pltpu.SemaphoreType.DMA
        pl.run_scoped(functools.partial(body, *refs),
                      dma((3,)), dma((RS,)), dma((1,)), dma((2,)), dma((2,)), dma((F // 128,)))

    def body(x_hbm, wr_hbm, gw_hbm, kt_hbm, vt_hbm, wq_hbm, wo_hbm, wg_hbm, wu_hbm, wd_hbm,
             out_ref,
             x_v, wr_v, gw_v, ring, wq_v, wo_v, wg_v, wu_v, wd_v, acc_s,
             ssem, rsem, qsem, osem, fsem, dsem):
        SK = kt_hbm.shape[-1]
        W = min(4096, max(256, SK // 4))
        NC = W // CW
        base = SK - W

        def mo(v, m):
            return v if isinstance(v, int) else pl.multiple_of(v, m)

        def loc(i):
            ph, r = divmod(i, NS * NC)
            if ph == 2:
                return ph, r % NS, r // NS
            blk, r = divmod(r, NS * BW)
            return ph, r // BW, blk * BW + r % BW

        def gm(g):
            return (g + goff) % NG

        def p1(g, i):
            g = gm(g)
            ph, s, c = loc(i)
            rows = pl.ds(s * SR, SR)
            if ph == 0:
                src = kt_hbm.at[g, rows, pl.ds(base + c * CW, CW)]
            elif ph == 1:
                src = vt_hbm.at[g, rows, pl.ds(base + c * CW, CW)]
            else:
                src = wo_hbm.at[pl.ds(g * GD + s * SR, SR), pl.ds(c * CW, CW)]
            return pltpu.make_async_copy(src, ring.at[i % RS], rsem.at[i % RS])

        def rect(src, dst, r0, nr, c0, nc, dr0, dc0, shp, sem):
            out = []
            pr, pc = shp
            for c in range(0, nc, pc):
                for r in range(0, nr, pr):
                    h = min(pr, nr - r)
                    w = min(pc, nc - c)

                    def mk(r=r, c=c, h=h, w=w):
                        d = dst.at[pl.ds(mo(dr0 + r, AL), h), pl.ds(mo(dc0 + c, 128), w)]
                        return pltpu.make_async_copy(
                            src.at[pl.ds(mo(r0 + r, AL), h), pl.ds(mo(c0 + c, 128), w)], d, sem), d
                    out.append(mk)
            return out

        def rect_rows(src, dst, r0, nr, nc, shp, sem, dr0=None):
            out = []
            for r in range(0, nr, shp[0]):
                out += rect(src, dst, r0 + r, min(shp[0], nr - r), 0, nc, (r0 if dr0 is None else dr0) + r, 0, shp, sem)
            return out

        def wq_pieces(g):
            g = gm(g)
            nb, pr, pc = pq3 if pq3 else (1,) + tuple(pq)
            idx = [(b, r, c) for b in range(0, QB, nb) for r in range(0, D // QB, pr) for c in range(0, GD, pc)]
            if qorder == 'r':
                idx.sort(key=lambda t: (t[2], t[0], t[1]))
            elif qorder == 'b':
                idx.sort(key=lambda t: (t[2], t[1], t[0]))
            out = []
            for b, r, c in idx:
                def mk(b=b, r=r, c=c):
                    h = min(pr, D // QB - r)
                    d = wq_v.at[pl.ds(b, nb), pl.ds(r, h), pl.ds(c, pc)]
                    return pltpu.make_async_copy(
                        wq_hbm.at[pl.ds(b, nb), pl.ds(r, h), pl.ds(mo(g * GD + c, 128), pc)], d, qsem.at[0]), d.at[0]
                out.append(mk)
            return out

        def wo_pieces(g):
            return rect_rows(wo_hbm, wo_v.at[g % 2], gm(g) * GD, GD, D, po, osem.at[g % 2], dr0=0)

        def gu_pieces(r0, nr):
            a = rect_rows(wg_hbm, wg_v, r0, nr, F, pf, fsem.at[0])
            b = rect_rows(wu_hbm, wu_v, r0, nr, F, pf, fsem.at[1])
            return [p for ab in zip(a, b) for p in ab]

        def wd_pieces():
            out = []
            for b in range(F // 128):
                out += rect_rows(wd_hbm, wd_v, b * 128, 128, D, pd, dsem.at[b])
            return out

        def wait_full(ref, sem):
            pltpu.make_async_copy(ref, ref, sem).wait()

        cx = pltpu.make_async_copy(x_hbm, x_v, ssem.at[0])
        cr = pltpu.make_async_copy(wr_hbm, wr_v, ssem.at[1])
        cg = pltpu.make_async_copy(gw_hbm, gw_v, ssem.at[2])

        sc = scope("pro"); sc.__enter__()
        p1(0, 0).start(priority=1)
        pltpu.make_async_copy(wq_hbm.at[:, :, pl.ds(gm(0) * GD, GD)], wq_v, qsem.at[0]).start(priority=0)
        cx.start()
        for i in range(1, D1):
            p1(0, i).start(priority=1)
        cr.start(); cg.start()

        row = lax.broadcasted_iota(jnp.int32, (8, GD), 0)
        col = lax.broadcasted_iota(jnp.int32, (8, GD), 1)
        diag = (col >= row * DH) & (col < (row + 1) * DH)
        scale = DH ** -0.5

        acc_s[...] = jnp.zeros_like(acc_s)
        wo_v[1] = jnp.zeros((GD, D), bf16)
        cx.wait()
        x8 = jnp.broadcast_to(x_v[...], (8, D))

        def q_tile(t):
            if not compute:
                return jnp.zeros((8, 128), bf16)
            qt = jnp.dot(x8, wq_v[:, :, t * 128:(t + 1) * 128].reshape(D, 128), preferred_element_type=f32)
            return jnp.where(diag[:, t * 128:(t + 1) * 128], qt, 0.0).astype(bf16)

        wait_full(wq_v, qsem.at[0])
        q0 = jnp.concatenate([q_tile(t) for t in range(NT)], axis=1)
        sc.__exit__(None, None, None)

        def assign(pieces_at, nunits):
            slots = [(u, k) for u in range(nunits) for k in use]
            sched = {}
            for lo, hi, ps in pieces_at:
                n = hi - lo
                for i, p in enumerate(ps):
                    sched.setdefault(slots[lo + (i * n) // len(ps)], []).append(p)
            return sched

        def group(g, q, on_prev, last):
            nunits = 2 * NC + (D // CW if last else 0)
            L = nunits * NS
            nsl = 2 * NC * len(use)
            if last:
                gu = gu_pieces(0, FR0)
                wd = wd_pieces()
                n1 = (len(gu) * (nsl - lastlim)) // (len(gu) + len(wd))
                sched = assign([(0, n1, gu), (n1, nsl - lastlim, wd)], nunits)
                wd_unit = {}
                per = len(wd) // (F // 128)
                for (u, k), ps in sched.items():
                    for p in ps:
                        if p in wd and wd.index(p) % per == per - 1:
                            wd_unit[wd.index(p) // per] = u
                HW = max(D // CW, LAG + max(u for (u, k), ps in sched.items() if any(p in gu for p in ps)))
            else:
                gu = gu_pieces(FR0 + g * FR, FR)
                m2 = min(n2, len(gu))
                wqp = wq_pieces(g + 1)
                wop = wo_pieces(g)
                seq = gu[:len(gu) - m2] + wop + wqp + gu[len(gu) - m2:]
                sched = assign([(0, nsl, seq)], nunits)
                QW = LAG + max(u for (u, k), ps in sched.items() if any(p in wqp for p in ps)) - NC
                assert 0 <= QW < NC
                assert max(u for (u, k), ps in sched.items() if any(p in wop for p in ps)) < 2 * NC - 1

            issued = []

            def issue(u, k, pin_val=None):
                for p in sched.get((u, k), []):
                    issued.append(p)
                    cp, dref = p()
                    if pin_val is not None:
                        pv = pin_val if AL == 8 else jnp.concatenate([pin_val, pin_val], axis=0)
                        dref[0:AL, 0:128] = pv.astype(bf16)
                    cp.start(priority=0)

            def ticks(u, lo=0, hi=NS):
                for s in range(lo, hi):
                    i = u * NS + s
                    p1(g, i).wait()
                    issue(u, s)
                    nxt = i + D1
                    if nxt < L:
                        p1(g, nxt).start(priority=1)
                    elif not last:
                        p1(g + 1, nxt - L).start(priority=1)

            slot_prev = (g + 1) % 2
            ss = [None] * NC
            mrun = None
            hs = []
            y = None
            ydone = 0
            stash = {}

            def extras(u):
                nonlocal y, ydone
                if not compute:
                    return
                if u < D // CW:
                    c = u
                    acc_s[:, c * CW:(c + 1) * CW] += jnp.dot(on_prev, wo_v[slot_prev, :, c * CW:(c + 1) * CW],
                                                             preferred_element_type=f32)
                if last:
                    if HW <= u < HW + F // 128:
                        c = u - HW
                        gg = jnp.dot(x8, wg_v[:, c * 128:(c + 1) * 128], preferred_element_type=f32)
                        uu = jnp.dot(x8, wu_v[:, c * 128:(c + 1) * 128], preferred_element_type=f32)
                        hs.append((gg * jax.nn.sigmoid(gg) * uu).astype(bf16))
                    elif stash.get("wd", 0) > ydone and len(hs) > ydone:
                        b = ydone
                        part = jnp.dot(hs[b], wd_v[b * 128:(b + 1) * 128, :], preferred_element_type=f32)
                        y = part if y is None else y + part
                        ydone += 1

            def waits(u):
                if last:
                    if u == HW:
                        assert all(p in issued for p in gu)
                        wait_full(wg_v, fsem.at[0])
                        wait_full(wu_v, fsem.at[1])
                    b = stash.get("wd", 0)
                    while b < F // 128 and u >= wd_unit[b] + LAG:
                        assert all(p in issued for p in wd[b * per:(b + 1) * per])
                        wait_full(wd_v.at[pl.ds(b * 128, 128), :], dsem.at[b])
                        b += 1
                    stash["wd"] = b
                else:
                    if u == NC + QW:
                        assert all(p in issued for p in wqp)
                        wait_full(wq_v, qsem.at[0])
                    if u == 2 * NC - 1:
                        assert all(p in issued for p in wop)
                        wait_full(wo_v.at[g % 2], osem.at[g % 2])

            sc = scope("K"); sc.__enter__()
            for u in range(NC):
                waits(u)
                ticks(u)
                if compute:
                    parts = []
                    for i in range(u * NS, (u + 1) * NS):
                        _, s, c = loc(i)
                        pp = [jnp.dot(q[:, s * SR + t * 128:s * SR + (t + 1) * 128], ring[i % RS, t * 128:(t + 1) * 128, :],
                                      preferred_element_type=f32) for t in range(TPS)]
                        parts += pp
                        if i == u * NS:
                            for k, t in enumerate(mids):
                                issue(u, NS + k, parts[t] if pin else None)
                        for x_ in pp:
                            ss[c] = x_ if ss[c] is None else ss[c] + x_
                        if s == NS - 1:
                            mrun = ss[c] if mrun is None else jnp.maximum(mrun, ss[c])
                else:
                    for k in range(len(mids)):
                        issue(u, NS + k)
                extras(u)
            sc.__exit__(None, None, None)
            sc = scope("V"); sc.__enter__()
            if compute:
                m = jnp.max(mrun, axis=-1, keepdims=True)
            o = [jnp.zeros((8, 128), f32) for _ in range(NT)]
            lrun = jnp.zeros((8, 128), f32)
            qn = []
            for j in range(NC):
                u = NC + j
                waits(u)
                ticks(u)
                if compute:
                    for i in range(u * NS, (u + 1) * NS):
                        _, s, c = loc(i)
                        if s == 0:
                            p = jnp.exp((ss[c] - m) * scale)
                            lrun = lrun + p
                            ss[c] = p.astype(bf16)
                        pp = [lax.dot_general(ss[c], ring[i % RS, t * 128:(t + 1) * 128, :], (((1,), (1,)), ((), ())),
                                              preferred_element_type=f32) for t in range(TPS)]
                        if i == u * NS:
                            for k, t in enumerate(mids):
                                issue(u, NS + k, pp[t] if pin else None)
                        for t in range(TPS):
                            o[s * TPS + t] = o[s * TPS + t] + pp[t]
                else:
                    for k in range(len(mids)):
                        issue(u, NS + k)
                if not last and j >= QW:
                    todo = NT - len(qn)
                    left = NC - j
                    for _ in range(-(-todo // left)):
                        qn.append(q_tile(len(qn)))
                extras(u)
            if compute:
                l = jnp.sum(lrun, axis=-1, keepdims=True)
                on = jnp.where(diag, jnp.concatenate(o, axis=1) / l, 0.0)
                if ft:
                    on = jnp.broadcast_to(jnp.sum(on, axis=0, keepdims=True), (8, GD))
                on = on.astype(bf16)
            else:
                on = on_prev
            sc.__exit__(None, None, None)
            if not last:
                assert len(issued) == len(seq)
                return jnp.concatenate(qn, axis=1), on
            sc = scope("tail"); sc.__enter__()

            cr.wait(); cg.wait()
            xf = x_v[...].astype(f32)
            wr = wr_v[...].astype(f32)
            gw = gw_v[...].astype(f32)
            r_acc = jnp.zeros((1, 128), f32)
            g_acc = jnp.zeros((1, 128), f32)
            for j in range(D // 128):
                xs = xf[:, j * 128:(j + 1) * 128]
                r_acc = r_acc + xs * wr[j:j + 1, :]
                g_acc = g_acc + xs * gw[j:j + 1, :]
            r_sel = jax.nn.sigmoid(jnp.sum(r_acc, axis=-1, keepdims=True))
            gate = jax.nn.sigmoid(jnp.sum(g_acc, axis=-1, keepdims=True))
            def wo_dot(u, lo, hi):
                r = None
                for s in range(lo, hi):
                    d = jnp.dot(on[:, s * SR:(s + 1) * SR], ring[(u * NS + s) % RS], preferred_element_type=f32)
                    r = d if r is None else r + d
                return r

            if ft and compute:
                NO = D // CW
                for c in range(NO - 1):
                    u = 2 * NC + c
                    waits(u)
                    ticks(u)
                    if c == NO - 2:
                        ticks(u + 1, 0, 1)
                    acc_s[:, c * CW:(c + 1) * CW] += wo_dot(u, 0, NS)
                    for k in range(len(mids)):
                        issue(u, NS + k)
                    while stash["wd"] > ydone:
                        extras(u)
                assert ydone == F // 128
                u = 2 * NC + NO - 1
                acc_s[:, D - CW:] += wo_dot(u, 0, 1)
                b = xf + (xf * 0.0 + y[0:1, :] * r_sel)
                pre = gate * acc_s[0:1, :]
                post = (1.0 - gate) * b
                out_ref[:, :D - CW] = (pre + post)[:, :D - CW].astype(out_ref.dtype)
                a_last = acc_s[0:1, D - CW:]
                post_last = post[:, D - CW:]
                ticks(u, 1, NS)
                a_last = a_last + wo_dot(u, 1, NS)[0:1, :]
                out_ref[:, D - CW:] = (gate * a_last + post_last).astype(out_ref.dtype)
                sc.__exit__(None, None, None)
                return
            res = []
            for c in range(D // CW):
                u = 2 * NC + c
                waits(u)
                ticks(u)
                if compute:
                    a = acc_s[:, c * CW:(c + 1) * CW] + wo_dot(u, 0, NS)
                    res.append(jnp.sum(a, axis=0, keepdims=True))
                for k in range(len(mids)):
                    issue(u, NS + k)
                if c < D // CW - 1:
                    while compute and stash["wd"] > ydone:
                        extras(u)
            assert stash["wd"] == F // 128
            if compute:
                assert ydone == F // 128
                b = xf + (xf * 0.0 + y[0:1, :] * r_sel)
                out_ref[...] = (gate * jnp.concatenate(res, axis=1) + (1.0 - gate) * b).astype(out_ref.dtype)
            else:
                out_ref[...] = (gate * xf).astype(out_ref.dtype)
            sc.__exit__(None, None, None)

        on0 = jnp.zeros((8, GD), bf16)
        qlast, onlast = lax.fori_loop(0, NG - 1, lambda g, c: group(g, c[0], c[1], False), (q0, on0))
        group(NG - 1, qlast, onlast, True)

    @jax.jit
    def pallas_gated_mix__sliding_block_cached__moe_arch_mod__decode_kernel(A_x, A_k_cache, A_v_cache, A_wq, A_wo, B_x, B_w_r, B_w_gate, B_w_up, B_w_down, gate_w):
        SK = A_k_cache.shape[2]
        kt = jnp.swapaxes(A_k_cache, 2, 3).reshape(NG, GD, SK)
        vt = jnp.swapaxes(A_v_cache, 2, 3).reshape(NG, GD, SK)
        x = A_x.reshape(1, D)
        wr = B_w_r.reshape(D // 128, 128)
        gw = gate_w.reshape(D // 128, 128)
        bf = jnp.bfloat16
        out = pl.pallas_call(
            kernel,
            out_shape=jax.ShapeDtypeStruct((1, D), bf),
            in_specs=[pl.BlockSpec(memory_space=pl.ANY)] * 10,
            out_specs=pl.BlockSpec(memory_space=pltpu.VMEM),
            scratch_shapes=[
                pltpu.VMEM((1, D), bf), pltpu.VMEM((D // 128, 128), bf), pltpu.VMEM((D // 128, 128), bf),
                pltpu.VMEM((RS, SR, CW), bf),
                pltpu.VMEM((QB, D // QB, GD), bf), pltpu.VMEM((2, GD, D), bf),
                pltpu.VMEM((D, F), bf), pltpu.VMEM((D, F), bf), pltpu.VMEM((F, D), bf),
                pltpu.VMEM((8, D), jnp.float32),
            ],
            compiler_params=pltpu.CompilerParams(vmem_limit_bytes=64 * 1024 * 1024, disable_bounds_checks=nobc),
        )(x, wr, gw, kt, vt, A_wq.reshape(QB, D // QB, H * DH), A_wo, B_w_gate, B_w_up, B_w_down)
        return out.reshape(1, 1, D)
    return pallas_gated_mix__sliding_block_cached__moe_arch_mod__decode_kernel


pallas_gated_mix__sliding_block_cached__moe_arch_mod__decode_kernel = _build(pin=True,AL=16,FR=80,po=(16,384),pf=(16,384),pd=(16,384),QB=1,pq=(32,128))
```

```python
import contextlib
import functools
import jax
import jax.numpy as jnp
from jax import lax
from jax.experimental import pallas as pl
from jax.experimental.pallas import tpu as pltpu

D = 640
H = 32
DH = 192
F = 1536
G = 4
NG = H // G
GD = G * DH
T = 128
HT = T // 2
NT = GD // T
CPU = 4
ND = D // T
NF = F // T
NB = 8
TR = 2 * T


def _build(D1=20, RS=32, compute=True, pq=(8, 768), pq0=(64, 128), qstep=7, qstep0=1, po=(8, 384), pf=(8, 512), pd=(8, 384),
          LAG=3, TPR=2, TPRV=2, pin=True, endlim=8, order="oqf", alt=True, osh=6, NTL=8, tsplit=(4, 6),
          use=(0, 1, 2, 3, 4), snake=True, nobc=True, scopes=False, fine=0):
    bf16 = jnp.bfloat16
    f32 = jnp.float32
    scope = jax.named_scope if scopes else (lambda name: contextlib.nullcontext())

    def kernel(*refs):
        dma = pltpu.SemaphoreType.DMA
        pl.run_scoped(functools.partial(body, *refs), dma((4,)), dma((RS,)), dma((NB,)))

    def body(x_hbm, wr_hbm, gw_hbm, kt_hbm, vt_hbm, wq_hbm, wo_hbm, wg_hbm, wu_hbm, wd_hbm,
             out_ref,
             x_v, wr_v, gw_v, ring, wq_v, wo_v, wg_v, wu_v, wd_v, qf_s, qr_s, acc_s, gu_s,
             ssem, rsem, bsem):
        SK = kt_hbm.shape[-1]
        W = min(4096, max(256, SK // 4))
        NC = W // T
        base = SK - W
        UP = G * NC // CPU
        UG = 2 * UP
        LM = NG * UG * CPU
        trects = [(H * DH - GD + r, c) for r in range(0, GD, TR) for c in range(0, D, T)][-NTL:]
        L = LM + len(trects)

        def loc(i):
            g, r = divmod(i, UG * CPU)
            ph, r = divmod(r, NC * G)
            s, c = divmod(r, NC)
            return g, ph, s, (NC - 1 - c if snake and s % 2 else c)

        def p1(i):
            if i >= LM:
                r, c = trects[i - LM]
                return pltpu.make_async_copy(wo_hbm.at[pl.ds(r, TR), pl.ds(c, T)], wo_v.at[pl.ds(r, TR), pl.ds(c, T)],
                                             rsem.at[i % RS])
            g, ph, s, c = loc(i)
            src = (kt_hbm, vt_hbm)[ph].at[g * G + s, :, pl.ds(base + c * T, T)]
            return pltpu.make_async_copy(src, ring.at[i % RS], rsem.at[i % RS])

        class Batch:
            def __init__(self, kind, idx, src, dst, r0, nr, c0, nc, shp, step=1):
                self.kind, self.idx = kind, idx
                self.src, self.dst = src, dst
                self.full = dst.at[pl.ds(r0, nr), pl.ds(c0, nc)]
                rects = [(r0 + r, min(shp[0], nr - r), c0 + c, min(shp[1], nc - c))
                         for r in range(0, nr, shp[0]) for c in range(0, nc, shp[1])]
                self.left = n = len(rects)
                self.rects = [rects[(i * step) % n] for i in range(n)]
                assert len(set(self.rects)) == n
                self.sem = None
                self.last_unit = None

            def pieces(self):
                return [(self, r) for r in self.rects]

        def b_q(t, n):
            return Batch("q", (t, n), wq_hbm, wq_v, 0, D, t * T, n * T, pq0 if t < NT else pq, qstep0 if t < NT else qstep)

        def o_cols(k):
            return min([D] + [c for r, c in trects if r <= k * T < r + TR])

        def b_o(k):
            return Batch("o", (k, o_cols(k)), wo_hbm, wo_v, k * T, T, 0, o_cols(k), po)

        fpieces = []
        for k in range(ND):
            a = Batch("g", (0, k), wg_hbm, wg_v, k * T, T, 0, F, pf).pieces()
            b = Batch("g", (1, k), wu_hbm, wu_v, k * T, T, 0, F, pf).pieces()
            fpieces += [p for ab in zip(a, b) for p in ab] if alt else a + b
        for k in range(NF):
            fpieces += Batch("d", k, wd_hbm, wd_v, k * T, T, 0, D, pd).pieces()
        first = [p for t in range(2, NT) for p in b_q(t, 1).pieces()]
        fixed = []
        for g in range(NG):
            qs = b_q((g + 1) * NT, NT).pieces() if g < NG - 1 else []
            lo, hi = max(0, g * NT - osh), ((g + 1) * NT - osh if g < NG - 1 else NG * NT)
            fixed.append((qs, [p for k in range(lo, hi) if o_cols(k) for p in b_o(k).pieces()]))

        def nbytes(ps):
            return sum(h * w for _, (r, h, c, w) in ps)

        total = nbytes(first) + nbytes(fpieces) + sum(nbytes(a) + nbytes(b) for a, b in fixed)
        seq = list(first)
        fpos = 0
        for g in range(NG):
            qs, os_ = fixed[g]
            room = (total * (g + 1)) // NG - nbytes(seq) - nbytes(qs) - nbytes(os_)
            f0 = fpos
            while fpos < len(fpieces) and (g == NG - 1 or nbytes(fpieces[f0:fpos + 1]) <= room):
                fpos += 1
            parts = dict(q=qs, o=os_, f=fpieces[f0:fpos])
            for ch in order:
                seq += parts[ch]
        assert nbytes(seq) == total
        slots = [(u, k) for u in range(NG * UG) for k in use]
        nsl = len(slots) - endlim
        sched = {}
        done = 0
        for p in seq:
            sz = nbytes([p])
            sl = slots[((2 * done + sz) * nsl) // (2 * total)]
            done += sz
            sched.setdefault(sl, []).append(p)
            p[0].last_unit = sl[0]

        sem_owner = [None] * NB
        pending = []

        def issue(u, k, pin_val=None):
            for b, (r, h, c, w) in sched.get((u, k), []):
                if b.sem is None:
                    b.sem = sem_owner.index(None)
                    sem_owner[b.sem] = b
                    pending.append(b)
                dst = b.dst.at[pl.ds(r, h), pl.ds(c, w)]
                if pin_val is not None:
                    dst[0:8, 0:T] = pin_val.astype(bf16)
                pltpu.make_async_copy(b.src.at[pl.ds(r, h), pl.ds(c, w)], dst, bsem.at[b.sem]).start(priority=0)
                b.left -= 1

        def ticks(lo, hi):
            for i in range(lo, hi):
                p1(i).wait()
                if i < LM:
                    issue(*divmod(i, CPU))
                if i + D1 < L:
                    p1(i + D1).start(priority=1)

        cx = pltpu.make_async_copy(x_hbm, x_v, ssem.at[0])
        cr = pltpu.make_async_copy(wr_hbm, wr_v, ssem.at[1])
        cg = pltpu.make_async_copy(gw_hbm, gw_v, ssem.at[2])
        cq = pltpu.make_async_copy(wq_hbm.at[:, pl.ds(0, 2 * T)], wq_v.at[:, pl.ds(0, 2 * T)], ssem.at[3])

        sc = scope("pro"); sc.__enter__()
        cx.start()
        cq.start(priority=0)
        for i in range(D1):
            p1(i).start(priority=1)
        cr.start(); cg.start()

        row = lax.broadcasted_iota(jnp.int32, (8, T), 0)
        low = lax.broadcasted_iota(jnp.int32, (8, T), 1) < HT
        high = jnp.logical_not(low)
        scale = DH ** -0.5

        acc_s[...] = jnp.zeros_like(acc_s)
        gu_s[...] = jnp.zeros_like(gu_s)
        cx.wait()
        x8 = jnp.broadcast_to(x_v[...], (8, D))
        xt = [x8[:, k * T:(k + 1) * T] for k in range(ND)]

        def mm(a, b):
            return jnp.dot(a, b, preferred_element_type=f32)

        def mmt(a, b):
            return lax.dot_general(a, b, (((1,), (1,)), ((), ())), preferred_element_type=f32)

        def swap(v):
            return jnp.concatenate([v[:, HT:], v[:, :HT]], axis=1)

        def collapse(v):
            return jnp.broadcast_to(jnp.sum(v, axis=0, keepdims=True), (8, T)).astype(bf16)

        def full(i, s):
            r = HT * (s % 2)
            return ring[i % RS, r:r + T, :]

        def rest(i, s):
            r = T * (1 - s % 2)
            return ring[i % RS, r:r + HT, :]

        q_ready = set()
        on = {}
        hs = []
        cnt = dict(g=0, d=0, o=0)
        tasks = []

        def add_tasks(b):
            if b.kind == "q":
                part = {}

                def fq(t, k, w):
                    d = mm(xt[k], w)
                    part[t] = part[t] + d if t in part else d
                    if k < ND - 1:
                        return
                    g, j = divmod(t, NT)
                    v = part[t]
                    if j % 3 == 1:
                        vs = swap(v)
                        for s, lo_, hi_ in ((2 * (j // 3), v, vs), (2 * (j // 3) + 1, vs, v)):
                            qr_s[g * G + s] = jnp.concatenate(
                                [jnp.where((row == s) & low, lo_, 0.0), jnp.where((row == s) & high, hi_, 0.0)],
                                axis=0).astype(bf16)
                    else:
                        s = 2 * (j // 3) + (j % 3) // 2
                        qf_s[g * G + s] = jnp.where(row == s, v, 0.0).astype(bf16)
                    q_ready.add(t)
                tasks.extend((0, functools.partial(fq, t, k), lambda: True, (wq_v, k, t))
                             for t in range(b.idx[0], b.idx[0] + b.idx[1]) for k in range(ND))
            elif b.kind == "o":
                k, nc = b.idx

                def fo(c, w):
                    acc_s[:, c * T:(c + 1) * T] += mm(on[k], w)
                    cnt["o"] += 1
                tasks.extend((1, functools.partial(fo, c), lambda: k in on, (wo_v, k, c)) for c in range(nc // T))
            elif b.kind == "g":
                m_, k = b.idx

                def fg(c, w):
                    gu_s[m_, :, c * T:(c + 1) * T] += mm(xt[k], w)
                    cnt["g"] += 1
                    if cnt["g"] == 2 * ND * NF:
                        gg = gu_s[0]
                        hh = (gg * jax.nn.sigmoid(gg) * gu_s[1]).astype(bf16)
                        hs.extend(hh[:, j * T:(j + 1) * T] for j in range(NF))
                        gu_s[0, :, 0:D] = jnp.zeros((8, D), f32)
                tasks.extend((1, functools.partial(fg, c), lambda: True, (b.dst, k, c)) for c in range(NF))
            else:
                k = b.idx

                def fd(c, w):
                    gu_s[0, :, c * T:(c + 1) * T] += mm(hs[k], w)
                    cnt["d"] += 1
                tasks.extend((2, functools.partial(fd, c), lambda: len(hs) > 0, (wd_v, k, c)) for c in range(ND))
            tasks.sort(key=lambda t_: t_[0])

        def waits(u):
            for b in list(pending):
                if b.left == 0 and u >= b.last_unit + LAG:
                    pltpu.make_async_copy(b.full, b.full, bsem.at[b.sem]).wait()
                    sem_owner[b.sem] = None
                    pending.remove(b)
                    if compute:
                        add_tasks(b)

        def side(n):
            while n:
                sel = [t_ for t_ in tasks if t_[2]()]
                if not sel:
                    return
                tasks.remove(sel[0])
                ref, r, c = sel[0][3]
                sel[0][1](ref[r * T:(r + 1) * T, c * T:(c + 1) * T])
                n -= 1

        def gates():
            cr.wait(); cg.wait()
            xf = x_v[...].astype(f32)
            wr = wr_v[...].astype(f32)
            gw = gw_v[...].astype(f32)
            r_acc = jnp.zeros((1, T), f32)
            g_acc = jnp.zeros((1, T), f32)
            for j in range(ND):
                xs = xf[:, j * T:(j + 1) * T]
                r_acc = r_acc + xs * wr[j:j + 1, :]
                g_acc = g_acc + xs * gw[j:j + 1, :]
            r_sel = jax.nn.sigmoid(jnp.sum(r_acc, axis=-1, keepdims=True))
            gate = jax.nn.sigmoid(jnp.sum(g_acc, axis=-1, keepdims=True))
            return xf, r_sel, gate

        cq.wait()
        if compute:
            add_tasks(Batch("q", (0, 2), wq_hbm, wq_v, 0, D, 0, 2 * T, (D, 2 * T)))
            side(2 * ND)
        sc.__exit__(None, None, None)

        def pairs(u):
            for i in range(u * CPU, (u + 1) * CPU, 2):
                _, _, s, c = loc(i)
                yield (s, c, i, i + 1) if c % 2 == 0 else (s, c - 1, i + 1, i)

        def add(a, b):
            return b if a is None else a + b

        for g in range(NG):
            ss = [None] * NC
            mrun = None
            sc = scope("K"); sc.__enter__()
            for j in range(UP):
                u = g * UG + j
                if fine and j and j % fine == 0:
                    sc.__exit__(None, None, None)
                    sc = scope(f"K{j}"); sc.__enter__()
                if g == NG - 1 and j == UP - 1:
                    xf, r_sel, gate = gates()
                waits(u)
                ticks(u * CPU, (u + 1) * CPU)
                if not compute:
                    issue(u, CPU)
                    continue
                side(TPR if g or j > 24 else max(TPR, 3))
                for n, (s, c, ie, io) in enumerate(pairs(u)):
                    k = g * NT + 3 * (s // 2)
                    assert k + 1 in q_ready and k + 2 * (s % 2) in q_ready, (g, j, s)
                    qf = qf_s[g * G + s]
                    de = mm(qf, full(ie, s))
                    if n == 0:
                        issue(u, CPU, de if pin else None)
                    do = mm(qf, full(io, s))
                    dr = mm(qr_s[g * G + s], jnp.concatenate([rest(ie, s), rest(io, s)], axis=0))
                    ss[c] = add(ss[c], de + dr[0:8])
                    ss[c + 1] = add(ss[c + 1], do + dr[8:16])
                    if s == G - 1:
                        mx = jnp.maximum(ss[c], ss[c + 1])
                        mrun = mx if mrun is None else jnp.maximum(mrun, mx)
            sc.__exit__(None, None, None)
            sc = scope("V"); sc.__enter__()
            if compute:
                m = jnp.max(mrun, axis=-1, keepdims=True)
            lrun = None
            of = oa = ob = mid = None
            for j in range(UP):
                u = g * UG + UP + j
                if fine and j and j % fine == 0:
                    sc.__exit__(None, None, None)
                    sc = scope(f"V{j}"); sc.__enter__()
                waits(u)
                ticks(u * CPU, (u + 1) * CPU)
                if not compute:
                    issue(u, CPU)
                    continue
                side(TPRV)
                for n, (s, c, ie, io) in enumerate(pairs(u)):
                    if s == 0:
                        pe = jnp.exp((ss[c] - m) * scale)
                        po_ = jnp.exp((ss[c + 1] - m) * scale)
                        lrun = add(lrun, pe + po_)
                        ss[c] = jnp.concatenate([pe, po_], axis=0).astype(bf16)
                    de = mmt(ss[c], full(ie, s))[0:8]
                    if n == 0:
                        issue(u, CPU, de if pin else None)
                    do = mmt(ss[c], full(io, s))[8:16]
                    dr = mmt(ss[c], jnp.concatenate([rest(ie, s), rest(io, s)], axis=0))
                    of = add(of, de + do)
                    oa = add(oa, dr[0:8])
                    ob = add(ob, dr[8:16])
                if (j + 1) % (NC // CPU) == 0:
                    if s == 0:
                        linv = 1.0 / jnp.sum(lrun, axis=-1, keepdims=True)
                    k = g * NT + 3 * (s // 2)
                    on[k + 2 * (s % 2)] = collapse(jnp.where(row == s, of * linv, 0.0))
                    if s % 2 == 0:
                        mid = jnp.where((row == s) & low, (oa + swap(ob)) * linv, 0.0)
                    else:
                        on[k + 1] = collapse(mid + jnp.where((row == s) & high, (ob + swap(oa)) * linv, 0.0))
                    of = oa = ob = None
            sc.__exit__(None, None, None)

        sc = scope("tail"); sc.__enter__()
        bounds = [0] + list(tsplit) + [len(trects)]
        U = NG * UG
        res = {}
        pre = None
        for n in range(len(bounds) - 1):
            waits(U + LAG if n == len(bounds) - 3 else U)
            ticks(LM + bounds[n], LM + bounds[n + 1])
            if not compute:
                continue
            side(len(tasks))
            for r, c in trects[bounds[n]:bounds[n + 1]]:
                d = mm(jnp.concatenate([on[r // T], on[r // T + 1]], axis=1), wo_v[r:r + TR, c:c + T])[0:1, :]
                res[c] = add(res.get(c), d)
            if pre is None and not pending and not tasks:
                assert cnt == dict(g=2 * ND * NF, d=ND * NF, o=NG * NT * ND - 2 * len(trects))
                post = (1.0 - gate) * (xf + (xf * 0.0 + gu_s[0, 0:1, 0:D] * r_sel))
                pre = {c: gate * acc_s[0:1, c:c + T] + post[:, c:c + T] for c in range(0, D, T)}
            for c in list(pre or ()):
                if all(c_ != c for _, c_ in trects[bounds[n + 1]:]):
                    v = pre.pop(c)
                    if c in res:
                        v = v + gate * res[c]
                    out_ref[:, c:c + T] = v.astype(out_ref.dtype)
        assert not pending and not tasks and all(b.left == 0 for b, _ in seq)
        if compute:
            assert pre == {}
        else:
            out_ref[...] = (gate * xf).astype(out_ref.dtype)
        sc.__exit__(None, None, None)

    @jax.jit
    def pallas_gated_mix__sliding_block_cached__moe_arch_mod__decode_kernel(A_x, A_k_cache, A_v_cache, A_wq, A_wo, B_x, B_w_r, B_w_gate, B_w_up, B_w_down, gate_w):
        SK = A_k_cache.shape[2]
        kt = jnp.swapaxes(A_k_cache, 2, 3).reshape(H, DH, SK)
        vt = jnp.swapaxes(A_v_cache, 2, 3).reshape(H, DH, SK)
        x = A_x.reshape(1, D)
        wr = B_w_r.reshape(ND, T)
        gw = gate_w.reshape(ND, T)
        bf = jnp.bfloat16
        out = pl.pallas_call(
            kernel,
            out_shape=jax.ShapeDtypeStruct((1, D), bf),
            in_specs=[pl.BlockSpec(memory_space=pl.ANY)] * 10,
            out_specs=pl.BlockSpec(memory_space=pltpu.VMEM),
            scratch_shapes=[
                pltpu.VMEM((1, D), bf), pltpu.VMEM((ND, T), bf), pltpu.VMEM((ND, T), bf),
                pltpu.VMEM((RS, DH, T), bf),
                pltpu.VMEM((D, H * DH), bf), pltpu.VMEM((H * DH, D), bf),
                pltpu.VMEM((D, F), bf), pltpu.VMEM((D, F), bf), pltpu.VMEM((F, D), bf),
                pltpu.VMEM((H, 8, T), bf), pltpu.VMEM((H, 16, T), bf),
                pltpu.VMEM((8, D), jnp.float32), pltpu.VMEM((2, 8, F), jnp.float32),
            ],
            compiler_params=pltpu.CompilerParams(vmem_limit_bytes=64 * 1024 * 1024, disable_bounds_checks=nobc),
        )(x, wr, gw, kt, vt, A_wq, A_wo, B_w_gate, B_w_up, B_w_down)
        return out.reshape(1, 1, D)
    return pallas_gated_mix__sliding_block_cached__moe_arch_mod__decode_kernel


pallas_gated_mix__sliding_block_cached__moe_arch_mod__decode_kernel = _build(use=(1, 3, 4))
```

```python
import contextlib
import functools
import jax
import jax.numpy as jnp
from jax import lax
from jax.experimental import pallas as pl
from jax.experimental.pallas import tpu as pltpu

D = 640
H = 32
DH = 192
F = 1536
G = 4
NG = H // G
GD = G * DH
T = 128
HT = T // 2
NT = GD // T
CPU = 4
ND = D // T
NF = F // T
NB = 8
TR = 2 * T


def _build(D1=20, RS=32, compute=True, pq=(8, 768), pq0=(32, 128), qstep=7, qstep0=3, po=(8, 384), pf=(8, 512), pd=(8, 384),
          LAG=3, TPR=2, TPRV=2, pin=True, endlim=2, order="of", alt=True, NTL=8, tsplit=(4, 6), NQ0=5, NPRE=4, NFE=20,
          use=(1, 3, 4), snake=True, unroll=False, nobc=True, scopes=False, fine=0):
    bf16 = jnp.bfloat16
    f32 = jnp.float32
    scope = jax.named_scope if scopes else (lambda name: contextlib.nullcontext())

    def kernel(*refs):
        dma = pltpu.SemaphoreType.DMA
        pl.run_scoped(functools.partial(body, *refs), dma((3 + NQ0,)), dma((RS,)), dma((NB,)), pltpu.SemaphoreType.REGULAR)

    def body(x_hbm, wr_hbm, gw_hbm, kt_hbm, vt_hbm, wq_hbm, wo_hbm, wg_hbm, wu_hbm, wd_hbm,
             out_ref,
             x_v, wr_v, gw_v, ring, wq_v, wo_v, wg_v, wu_v, wd_v, xs_s, qf_s, qr_s, on_s, acc_s, gu_s,
             ssem, rsem, bsem, fence):
        SK = kt_hbm.shape[-1]
        W = min(4096, max(256, SK // 4))
        NC = W // T
        base = SK - W
        UP = G * NC // CPU
        UG = 2 * UP
        LG = UG * CPU
        assert LG % RS == 0 and RS - D1 >= CPU
        trects = [(r, c) for r in range(0, GD, TR) for c in range(0, D, T)][-NTL:]

        def mo(v, m):
            return v if isinstance(v, int) else pl.multiple_of(v, m)

        def is_last(g):
            return isinstance(g, int) and g == NG - 1

        def loc(i):
            ph, r = divmod(i, NC * G)
            s, c = divmod(r, NC)
            return ph, s, (NC - 1 - c if snake and s % 2 else c)

        def p1(g, i):
            if i >= LG and is_last(g):
                r, c = trects[i - LG]
                return pltpu.make_async_copy(wo_hbm.at[pl.ds(g * GD + r, TR), pl.ds(c, T)],
                                             wo_v.at[1, pl.ds(r, TR), pl.ds(c, T)], rsem.at[i % RS])
            if i >= LG:
                g, i = g + 1, i - LG
            ph, s, c = loc(i)
            src = (kt_hbm, vt_hbm)[ph].at[g * G + s, :, pl.ds(base + c * T, T)]
            return pltpu.make_async_copy(src, ring.at[i % RS], rsem.at[i % RS])

        class Batch:
            def __init__(self, kind, idx, key, src, r0, c0, dst, d0, e0, nr, nc, shp, step=1):
                self.kind, self.idx, self.key = kind, idx, (kind, key)
                self.src, self.r0, self.c0 = src, r0, c0
                self.dst = dst.at[pl.ds(d0, nr), pl.ds(e0, nc)]
                rects = [(r, min(shp[0], nr - r), c, min(shp[1], nc - c))
                         for r in range(0, nr, shp[0]) for c in range(0, nc, shp[1])]
                self.left = n = len(rects)
                self.rects = [rects[(i * step) % n] for i in range(n)]
                assert len(set(self.rects)) == n
                self.sem = None
                self.last_unit = None

            def pieces(self):
                return [(self, r) for r in self.rects]

        def b_q(g, t0=0, n=NT):
            buf = min(g, 2) if isinstance(g, int) else 2
            shp, step = (pq, qstep) if n == NT else (pq0, qstep0)
            return Batch("q", (g, t0, n), (buf, t0), wq_hbm, 0, g * GD + t0 * T, wq_v.at[buf], 0, t0 * T, D, n * T, shp, step)

        def b_o(g):
            out = []
            for k in range(NT):
                nc = min([D] + [c for r, c in trects if is_last(g) and r <= k * T < r + TR])
                if nc:
                    out += Batch("o", (is_last(g), k), (is_last(g), k), wo_hbm, g * GD + k * T, 0, wo_v.at[int(is_last(g))], k * T, 0,
                                 T, nc, po).pieces()
            return out

        def b_gu(k):
            a = Batch("g", (0, k), 0, wg_hbm, k * T, 0, wg_v, 0, 0, T, F, pf).pieces()
            b = Batch("g", (1, k), 1, wu_hbm, k * T, 0, wu_v, 0, 0, T, F, pf).pieces()
            return [p for ab in zip(a, b) for p in ab] if alt else a + b

        def b_d():
            return [p for k in range(NF) for p in Batch("d", k, k, wd_hbm, k * T, 0, wd_v, k * T, 0, T, D, pd).pieces()]

        sched = {}
        sem_owner = [None] * NB
        pending = []

        def plan(seq, slots):
            sched.clear()
            total = sum(h * w for _, (r, h, c, w) in seq)
            done = 0
            for p in seq:
                sz = p[1][1] * p[1][3]
                sl = slots[((2 * done + sz) * len(slots)) // (2 * total)]
                done += sz
                sched.setdefault(sl, []).append(p)
                p[0].last_unit = sl[0]

        tasks = []

        def claim(b):
            b.sem = 0 if b.key == ("q", (2, 0)) else sem_owner.index(None, 1)
            assert sem_owner[b.sem] is None
            assert all(o.key != b.key for o in pending) and all(t_[3].key != b.key for t_ in tasks)
            sem_owner[b.sem] = b
            pending.append(b)

        def issue(u, k, pin_val=None):
            for b, (r, h, c, w) in sched.pop((u, k), []):
                if b.sem is None:
                    claim(b)
                dst = b.dst.at[pl.ds(r, h), pl.ds(c, w)]
                if pin_val is not None:
                    dst[0:8, 0:T] = pin_val.astype(bf16)
                src = b.src.at[pl.ds(mo(b.r0 + r, 8), h), pl.ds(mo(b.c0 + c, T), w)]
                pltpu.make_async_copy(src, dst, bsem.at[b.sem]).start(priority=0)
                b.left -= 1

        def ticks(g, u0, lo, hi):
            for i in range(lo, hi):
                p1(g, i).wait()
                if i < LG:
                    issue(u0 + i // CPU, i % CPU)
                if not is_last(g) or i + D1 < LG + len(trects):
                    p1(g, i + D1).start(priority=1)

        def barrier():
            pl.semaphore_signal(fence, 1)
            pl.semaphore_wait(fence, 1)

        def unit_slots(n):
            return [(u, k) for u in range(n) for k in use]

        cx = pltpu.make_async_copy(x_hbm, x_v, ssem.at[0])
        cr = pltpu.make_async_copy(wr_hbm, wr_v, ssem.at[1])
        cg = pltpu.make_async_copy(gw_hbm, gw_v, ssem.at[2])
        cq = [pltpu.make_async_copy(wq_hbm.at[pl.ds(k * (D // NQ0), D // NQ0), pl.ds(0, 2 * T)],
                                    wq_v.at[0, pl.ds(k * (D // NQ0), D // NQ0), pl.ds(0, 2 * T)], ssem.at[3 + k])
              for k in range(NQ0)]

        sc = scope("pro"); sc.__enter__()
        plan([p for t in range(2, NT) for p in b_q(0, t, 1).pieces()] + b_q(1).pieces() + b_q(2).pieces(),
             [(-2, k) for k in range(NPRE)] + [(-1, k) for k in range(NQ0)] + unit_slots(UG))
        cx.start()
        for c_ in cq:
            c_.start(priority=1)
        barrier()
        for i in range(D1):
            p1(0, i).start(priority=1)
        cr.start(); cg.start()
        for k in range(NPRE):
            for _ in range(NFE if k else 1):
                barrier()
            issue(-2, k)

        row = lax.broadcasted_iota(jnp.int32, (8, T), 0)
        low = lax.broadcasted_iota(jnp.int32, (8, T), 1) < HT
        high = jnp.logical_not(low)
        scale = DH ** -0.5

        acc_s[...] = jnp.zeros_like(acc_s)
        gu_s[...] = jnp.zeros_like(gu_s)
        cx.wait()
        x8 = jnp.broadcast_to(x_v[...], (8, D))
        for k in range(ND):
            xs_s[k] = x8[:, k * T:(k + 1) * T]

        def mm(a, b):
            return jnp.dot(a, b, preferred_element_type=f32)

        def mmt(a, b):
            return lax.dot_general(a, b, (((1,), (1,)), ((), ())), preferred_element_type=f32)

        def swap(v):
            return jnp.concatenate([v[:, HT:], v[:, :HT]], axis=1)

        def collapse(v):
            return jnp.broadcast_to(jnp.sum(v, axis=0, keepdims=True), (8, T)).astype(bf16)

        def add(a, b):
            return b if a is None else a + b

        def full(i, s):
            r = HT * (s % 2)
            return ring[i % RS, r:r + T, :]

        def rest(i, s):
            r = T * (1 - s % 2)
            return ring[i % RS, r:r + HT, :]

        q0_ready = set()
        on = {}
        hs = []

        def add_tasks(b):
            if b.kind == "q":
                g, t0, n = b.idx
                part = {}

                def fq(j, k):
                    part[j] = add(part.get(j), mm(xs_s[k], b.dst[k * T:(k + 1) * T, (j - t0) * T:(j - t0 + 1) * T]))
                    if k < ND - 1:
                        return
                    v = part[j]
                    if j % 3 == 1:
                        vs = swap(v)
                        for s, lo_, hi_ in ((2 * (j // 3), v, vs), (2 * (j // 3) + 1, vs, v)):
                            qr_s[g * G + s] = jnp.concatenate(
                                [jnp.where((row == s) & low, lo_, 0.0), jnp.where((row == s) & high, hi_, 0.0)],
                                axis=0).astype(bf16)
                    else:
                        s = 2 * (j // 3) + (j % 3) // 2
                        qf_s[g * G + s] = jnp.where(row == s, v, 0.0).astype(bf16)
                    if n < NT:
                        q0_ready.add(j)
                tasks.extend((0, functools.partial(fq, j, k), lambda: True, b)
                             for j in range(t0, t0 + n) for k in range(ND))
            elif b.kind == "o":
                last, k = b.idx

                def fo(c):
                    acc_s[:, c * T:(c + 1) * T] += mm(on[k] if last else on_s[k], b.dst[:, c * T:(c + 1) * T])
                tasks.extend((1, functools.partial(fo, c), lambda: not last or k in on, b)
                             for c in range(b.dst.shape[1] // T))
            elif b.kind == "g":
                m_, k = b.idx

                def fg(c):
                    gu_s[m_, :, c * T:(c + 1) * T] += mm(xs_s[k], b.dst[:, c * T:(c + 1) * T])
                tasks.extend((1, functools.partial(fg, c), lambda: True, b) for c in range(NF))
            else:
                k = b.idx

                def fd(c):
                    gu_s[0, :, c * T:(c + 1) * T] += mm(hs[k], b.dst[:, c * T:(c + 1) * T])
                tasks.extend((2, functools.partial(fd, c), lambda: True, b) for c in range(ND))
            tasks.sort(key=lambda t_: t_[0])

        def waits(u):
            for b in list(pending):
                if b.left == 0 and u >= b.last_unit + LAG:
                    pltpu.make_async_copy(b.dst, b.dst, bsem.at[b.sem]).wait()
                    sem_owner[b.sem] = None
                    pending.remove(b)
                    if compute:
                        add_tasks(b)

        def side(n):
            while n:
                sel = [t_ for t_ in tasks if t_[2]()]
                if not sel:
                    return
                tasks.remove(sel[0])
                sel[0][1]()
                n -= 1

        def live():
            return [b for ps in sched.values() for b, _ in ps] + pending + [t_[3] for t_ in tasks]

        def gates():
            cr.wait(); cg.wait()
            xf = x_v[...].astype(f32)
            wr = wr_v[...].astype(f32)
            gw = gw_v[...].astype(f32)
            r_acc = jnp.zeros((1, T), f32)
            g_acc = jnp.zeros((1, T), f32)
            for j in range(ND):
                xs = xf[:, j * T:(j + 1) * T]
                r_acc = r_acc + xs * wr[j:j + 1, :]
                g_acc = g_acc + xs * gw[j:j + 1, :]
            r_sel = jax.nn.sigmoid(jnp.sum(r_acc, axis=-1, keepdims=True))
            gate = jax.nn.sigmoid(jnp.sum(g_acc, axis=-1, keepdims=True))
            return xf, r_sel, gate

        for k, c_ in enumerate(cq):
            c_.wait()
            issue(-1, k)
        if compute:
            add_tasks(b_q(0, 0, 2))
        sc.__exit__(None, None, None)

        def pairs(j):
            for i in range(j * CPU, (j + 1) * CPU, 2):
                _, s, c = loc(i)
                yield (s, c, i, i + 1) if c % 2 == 0 else (s, c - 1, i + 1, i)

        def group(g, u0, hook=None):
            first = isinstance(g, int) and g == 0
            ss = [None] * NC
            mrun = None
            sc = scope("K"); sc.__enter__()
            for j in range(UP):
                u = u0 + j
                if fine and j and j % fine == 0:
                    sc.__exit__(None, None, None)
                    sc = scope(f"K{j}"); sc.__enter__()
                waits(u)
                ticks(g, u0, j * CPU, (j + 1) * CPU)
                if hook:
                    hook(j)
                if not compute:
                    issue(u, CPU)
                    continue
                side(TPR if not first or j > 24 else 2 * ND if j == 0 else max(TPR, 3))
                for n, (s, c, ie, io) in enumerate(pairs(j)):
                    assert not first or {3 * (s // 2) + 1, 3 * (s // 2) + 2 * (s % 2)} <= q0_ready, (j, s)
                    qf = qf_s[g * G + s]
                    de = mm(qf, full(ie, s))
                    if n == 0:
                        issue(u, CPU, de if pin else None)
                    do = mm(qf, full(io, s))
                    dr = mm(qr_s[g * G + s], jnp.concatenate([rest(ie, s), rest(io, s)], axis=0))
                    ss[c] = add(ss[c], de + dr[0:8])
                    ss[c + 1] = add(ss[c + 1], do + dr[8:16])
                    if s == G - 1:
                        mx = jnp.maximum(ss[c], ss[c + 1])
                        mrun = mx if mrun is None else jnp.maximum(mrun, mx)
            sc.__exit__(None, None, None)
            sc = scope("V"); sc.__enter__()
            if compute:
                m = jnp.max(mrun, axis=-1, keepdims=True)
            lrun = None
            of = oa = ob = mid = None

            def put(k, v):
                if is_last(g):
                    on[k] = v
                else:
                    assert not any(b.kind == "o" and b.stale for b in live())
                    on_s[k] = v

            for j in range(UP, UG):
                u = u0 + j
                if fine and j > UP and j % fine == 0:
                    sc.__exit__(None, None, None)
                    sc = scope(f"V{j}"); sc.__enter__()
                waits(u)
                ticks(g, u0, j * CPU, (j + 1) * CPU)
                if not compute:
                    issue(u, CPU)
                    continue
                side(TPRV)
                for n, (s, c, ie, io) in enumerate(pairs(j)):
                    if s == 0:
                        pe = jnp.exp((ss[c] - m) * scale)
                        po_ = jnp.exp((ss[c + 1] - m) * scale)
                        lrun = add(lrun, pe + po_)
                        ss[c] = jnp.concatenate([pe, po_], axis=0).astype(bf16)
                    de = mmt(ss[c], full(ie, s))[0:8]
                    if n == 0:
                        issue(u, CPU, de if pin else None)
                    do = mmt(ss[c], full(io, s))[8:16]
                    dr = mmt(ss[c], jnp.concatenate([rest(ie, s), rest(io, s)], axis=0))
                    of = add(of, de + do)
                    oa = add(oa, dr[0:8])
                    ob = add(ob, dr[8:16])
                if (j + 1) % (NC // CPU) == 0:
                    if s == 0:
                        linv = 1.0 / jnp.sum(lrun, axis=-1, keepdims=True)
                    k = 3 * (s // 2)
                    put(k + 2 * (s % 2), collapse(jnp.where(row == s, of * linv, 0.0)))
                    if s % 2 == 0:
                        mid = jnp.where((row == s) & low, (oa + swap(ob)) * linv, 0.0)
                    else:
                        put(k + 1, collapse(mid + jnp.where((row == s) & high, (ob + swap(oa)) * linv, 0.0)))
                    of = oa = ob = None
            sc.__exit__(None, None, None)

        def handover(g):
            assert not sched and not tasks and len(pending) == 1
            old = pending.pop()
            assert old.kind == "q" and old.left == 0 and old.sem == 0 and old.last_unit == UG - 1
            sem_owner[0] = None
            if g is not None:
                b = b_q(g)
                b.left, b.last_unit = 0, -1
                claim(b)

        Batch.stale = True
        group(0, 0)

        def middle(g, carry):
            handover(g + 1)
            parts = dict(o=b_o(g - 1), f=b_gu(g - 1))
            plan([p for ch in order for p in parts[ch]] + b_q(g + 2).pieces(), unit_slots(UG))
            group(g, 0)
            return carry

        if unroll:
            for g in range(1, ND + 1):
                middle(g, 0)
        else:
            lax.fori_loop(1, ND + 1, middle, 0)
        handover(NG - 1)
        o6 = b_o(NG - 2)
        for b, _ in o6:
            b.stale = False
        o7 = b_o(NG - 1)
        for b, _ in o7:
            b.stale = False
        plan(b_o(NG - 3) + b_d() + o6 + o7, unit_slots(2 * UG)[:2 * UG * len(use) - endlim])
        assert min(u for (u, _), ps in sched.items() if any(p in o6 for p in ps)) >= UG - LAG

        def swiglu(j):
            if j == 1 and compute:
                gg = gu_s[0]
                hh = (gg * jax.nn.sigmoid(gg) * gu_s[1]).astype(bf16)
                hs.extend(hh[:, k * T:(k + 1) * T] for k in range(NF))
                gu_s[0, :, 0:D] = jnp.zeros((8, D), f32)

        gv = []

        def scalars(j):
            if j == UP - 1:
                gv.extend(gates())

        group(NG - 2, 0, swiglu)
        assert not any(b.kind == "q" for b in live())
        group(NG - 1, UG, scalars)
        xf, r_sel, gate = gv

        sc = scope("tail"); sc.__enter__()
        bounds = [0] + list(tsplit) + [len(trects)]
        res = {}
        pre = None
        for n in range(len(bounds) - 1):
            ticks(NG - 1, UG, LG + bounds[n], LG + bounds[n + 1])
            waits(2 * UG + (LAG if n == len(bounds) - 3 else 0))
            if not compute:
                continue
            side(len(tasks))
            for r, c in trects[bounds[n]:bounds[n + 1]]:
                d = mm(jnp.concatenate([on[r // T], on[r // T + 1]], axis=1), wo_v[1, r:r + TR, c:c + T])[0:1, :]
                res[c] = add(res.get(c), d)
            if pre is None and not pending and not tasks:
                post = (1.0 - gate) * (xf + (xf * 0.0 + gu_s[0, 0:1, 0:D] * r_sel))
                pre = {c: gate * acc_s[0:1, c:c + T] + post[:, c:c + T] for c in range(0, D, T)}
            for c in list(pre or ()):
                if all(c_ != c for _, c_ in trects[bounds[n + 1]:]):
                    v = pre.pop(c)
                    if c in res:
                        v = v + gate * res[c]
                    out_ref[:, c:c + T] = v.astype(out_ref.dtype)
        assert not pending and not tasks and not sched
        if compute:
            assert pre == {}
        else:
            out_ref[...] = (gate * xf).astype(out_ref.dtype)
        sc.__exit__(None, None, None)

    @jax.jit
    def pallas_gated_mix__sliding_block_cached__moe_arch_mod__decode_kernel(A_x, A_k_cache, A_v_cache, A_wq, A_wo, B_x, B_w_r, B_w_gate, B_w_up, B_w_down, gate_w):
        SK = A_k_cache.shape[2]
        kt = jnp.swapaxes(A_k_cache, 2, 3).reshape(H, DH, SK)
        vt = jnp.swapaxes(A_v_cache, 2, 3).reshape(H, DH, SK)
        x = A_x.reshape(1, D)
        wr = B_w_r.reshape(ND, T)
        gw = gate_w.reshape(ND, T)
        bf = jnp.bfloat16
        out = pl.pallas_call(
            kernel,
            out_shape=jax.ShapeDtypeStruct((1, D), bf),
            in_specs=[pl.BlockSpec(memory_space=pl.ANY)] * 10,
            out_specs=pl.BlockSpec(memory_space=pltpu.VMEM),
            scratch_shapes=[
                pltpu.VMEM((1, D), bf), pltpu.VMEM((ND, T), bf), pltpu.VMEM((ND, T), bf),
                pltpu.VMEM((RS, DH, T), bf),
                pltpu.VMEM((3, D, GD), bf), pltpu.VMEM((2, GD, D), bf),
                pltpu.VMEM((T, F), bf), pltpu.VMEM((T, F), bf), pltpu.VMEM((F, D), bf),
                pltpu.VMEM((ND, 8, T), bf), pltpu.VMEM((H, 8, T), bf), pltpu.VMEM((H, 16, T), bf),
                pltpu.VMEM((NT, 8, T), bf),
                pltpu.VMEM((8, D), jnp.float32), pltpu.VMEM((2, 8, F), jnp.float32),
            ],
            compiler_params=pltpu.CompilerParams(vmem_limit_bytes=64 * 1024 * 1024, disable_bounds_checks=nobc),
        )(x, wr, gw, kt, vt, A_wq, A_wo, B_w_gate, B_w_up, B_w_down)
        return out.reshape(1, 1, D)
    return pallas_gated_mix__sliding_block_cached__moe_arch_mod__decode_kernel


pallas_gated_mix__sliding_block_cached__moe_arch_mod__decode_kernel = _build()
```
